```python
import os as _os
_os.environ.setdefault("JAX_PLATFORMS", "cpu")
import jax
import jax.numpy as jnp

def _softmax(x, axis=-1):
    return jax.nn.softmax(x, axis=axis)
def _gelu(x):
    return jax.nn.gelu(x, approximate=True)
def _silu(x):
    return jax.nn.silu(x)
def _sigmoid(x):
    return jax.nn.sigmoid(x)
def _layernorm(x, axis=-1, eps=1e-5):
    m = jnp.mean(x, axis=axis, keepdims=True)
    v = jnp.var(x, axis=axis, keepdims=True)
    return (x - m) / jnp.sqrt(v + eps)
def _scatter_add(tgt, idx, src, axis=0):
    return tgt.at[idx].add(src)
def _segment_sum(src, seg, n):
    return jax.ops.segment_sum(src, seg, n)
class _Rng:
    def __init__(self, key):
        self._k = key
    def _next(self):
        self._k, sub = jax.random.split(self._k)
        return sub
    def normal(self, shape):
        return jax.random.normal(self._next(), shape, dtype=jnp.bfloat16)
    def randint(self, lo, hi, shape):
        return jax.random.randint(self._next(), shape, lo, hi, dtype=jnp.int32)
    def uniform(self, shape, lo=0.0, hi=1.0):
        return jax.random.uniform(self._next(), shape, jnp.bfloat16, lo, hi)
    def permutation(self, n):
        return jax.random.permutation(self._next(), n)


kernel_name = 'sequential_preLN__mha_block__dense_activation_squared_relu__prompt'

def setup_inputs():
    _rng = _Rng(jax.random.key(int.from_bytes(__import__("os").urandom(4), "little")))
    _w = (lambda a: (lambda t: t.astype(jnp.bfloat16) if jnp.issubdtype(t.dtype, jnp.floating) else t)(jnp.asarray(a)))
    def _A_setup():
        B, S, D, H = 1, 2048, 448, 16
        return {
            "x": _w((lambda *s: _rng.normal(s) * 0.05)(B, S, D)),
            "wqkv": _w((lambda *s: _rng.normal(s) * 0.05)(D, 3 * D)),
            "wo": _w((lambda *s: _rng.normal(s) * 0.05)(D, D)),
        }
    _A_in = _A_setup()

    def _B_setup():
        B, S, D, F = 1, 2048, 448, 1792
        return {
            "x": _w((lambda *s: _rng.normal(s) * 0.05)(B, S, D)),
            "w1": _w((lambda *s: _rng.normal(s) * 0.05)(D, F)),
            "b1": _w((lambda *s: _rng.normal(s) * 0.05)(F)),
            "w2": _w((lambda *s: _rng.normal(s) * 0.05)(F, D)),
            "b2": _w((lambda *s: _rng.normal(s) * 0.05)(D)),
        }
    _B_in = _B_setup()

    return {
        "A_x": _A_in["x"],
        "A_wqkv": _A_in["wqkv"],
        "A_wo": _A_in["wo"],
        "B_x": _B_in["x"],
        "B_w1": _B_in["w1"],
        "B_b1": _B_in["b1"],
        "B_w2": _B_in["w2"],
        "B_b2": _B_in["b2"],
    }

def reference(A_x, A_wqkv, A_wo, B_x, B_w1, B_b1, B_w2, B_b2):
    def _A_ref(x, wqkv, wo):
        B, S, D = x.shape
        H = 16
        Dh = D // H
        qkv = (lambda x, *d: x.transpose(*d))((x @ wqkv).reshape(B, S, 3, H, Dh), 2, 0, 3, 1, 4)
        q, k, v = qkv[0], qkv[1], qkv[2]
        scores = jnp.einsum("bhqd,bhkd->bhqk", q, k) * (Dh ** -0.5)
        p = _softmax(scores, axis=-1)
        o = jnp.einsum("bhqk,bhkd->bhqd", p, v)
        return (lambda x, *d: x.transpose(*d))(o, 0, 2, 1, 3).reshape(B, S, D) @ wo

    def _B_ref(x, w1, b1, w2, b2):
        h = jnp.einsum("bsd,df->bsf", x, w1) + b1
        zero = jnp.zeros_like(h)
        r = jnp.where(h > zero, h, zero)
        h = r * r
        out = jnp.einsum("bsf,fd->bsd", h, w2) + b2
        return out

    x = A_x
    h = x + _A_ref(_layernorm(x, axis=-1), A_wqkv, A_wo)
    h2 = h + _B_ref(_layernorm(h, axis=-1), B_w1, B_b1, B_w2, B_b2)
    return h2
```

```python
import functools
import math

import jax
import jax.numpy as jnp
from jax import lax
import jax.experimental.pallas as pl
import jax.experimental.pallas.tpu as pltpu

bf16 = jnp.bfloat16
f32 = jnp.float32

S = 2048
D = 448
H = 16
DH = 28
F = 1792
G = 4
GW = G * DH
EPS = 1e-5
QSCALE = (DH ** -0.5) * math.log2(math.e)


def _ln_T(xt):
    mu = jnp.sum(xt, axis=0, keepdims=True) * (1.0 / D)
    xc = xt - mu
    var = jnp.sum(xc * xc, axis=0, keepdims=True) * (1.0 / D)
    return xc * lax.rsqrt(var + EPS)


def make_kernel(T1=256, TQ=256, KC=256, UNR=4, T3=256, SK=2, P1UNROLL=True, XSPLIT=512):
    NQ = S // TQ
    NU = NQ * H
    NC = S // KC
    N3 = S // T3

    def kern(xt_hbm, wqkv_hbm, wo_hbm, w1_hbm, b1_ref, w2t_hbm, b2_ref, out_hbm,
             xt_s, wqkv_s, wo_s, w1_s, w2T_s, wqkvT_s, woT_s, w1T_s, b1c_s, b2c_s,
             k_s, qt_s, vt_s, ot_s, sA, sB, y_s, in_sem, out_sem):
        cp_x0 = pltpu.make_async_copy(xt_hbm.at[:, pl.ds(0, XSPLIT)], xt_s.at[:, pl.ds(0, XSPLIT)], in_sem.at[0])
        cp_wqkv = pltpu.make_async_copy(wqkv_hbm, wqkv_s, in_sem.at[1])
        cp_x1 = pltpu.make_async_copy(xt_hbm.at[:, pl.ds(XSPLIT, S - XSPLIT)], xt_s.at[:, pl.ds(XSPLIT, S - XSPLIT)], in_sem.at[2])
        cp_wo = pltpu.make_async_copy(wo_hbm, wo_s, in_sem.at[3])
        cp_w1 = pltpu.make_async_copy(w1_hbm, w1_s, in_sem.at[4])
        cp_w2 = pltpu.make_async_copy(w2t_hbm, w2T_s, in_sem.at[5])
        cp_wqkv.start()
        cp_x0.start()
        cp_x1.start()
        cp_wqkv.wait()
        cp_x0.wait()
        cp_wo.start()
        cp_w1.start()
        cp_w2.start()

        wqkvT_s[...] = wqkv_s[...].T

        tail = (lax.broadcasted_iota(jnp.int32, (4, T1), 0) == 0).astype(f32)

        def p1(t):
            c0 = t * T1
            xt = xt_s[:, pl.ds(c0, T1)]
            xn = _ln_T(xt.astype(f32)).astype(bf16)
            kk = jnp.dot(wqkvT_s[D:2 * D, :], xn, preferred_element_type=f32)
            for g in range(G):
                kt = kk[g * GW:(g + 1) * GW].astype(bf16)
                k_s[g, pl.ds(c0, T1), :] = kt.T
            vv = jnp.dot(wqkvT_s[2 * D:3 * D, :], xn, preferred_element_type=f32)
            for h in range(H):
                v = vv[h * DH:(h + 1) * DH]
                vt_s[h * 32:(h + 1) * 32, pl.ds(c0, T1)] = jnp.concatenate([v, tail], axis=0).astype(bf16)
            qq = jnp.dot(wqkvT_s[0:D, :], xn, preferred_element_type=f32)
            qt_s[:, pl.ds(c0, T1)] = (qq * QSCALE).astype(bf16)

        for t in range(S // T1):
            if t * T1 == XSPLIT:
                cp_x1.wait()
            p1(t)

        row = lax.broadcasted_iota(jnp.int32, (GW, TQ), 0)

        def qweights(u):
            qt = u // H; h = u % H
            g = h // G; j = h % G
            if isinstance(u, int):
                q = qt_s[g * GW:(g + 1) * GW, qt * TQ:(qt + 1) * TQ]
            else:
                q = qt_s[pl.ds(pl.multiple_of(g * GW, 16), GW), pl.ds(pl.multiple_of(qt * TQ, TQ), TQ)]
            msk = (row >= j * DH) & (row < j * DH + DH)
            return jnp.where(msk, q, jnp.zeros_like(q)), g

        def qk_chunk(qwg, c, s_ref, m8):
            qw, g = qwg
            kc = k_s[g, pl.ds(c * KC, KC), :]
            s = jnp.dot(kc, qw, preferred_element_type=f32)
            s_ref[pl.ds(c * KC, KC), :] = s
            sm = jnp.max(s.reshape(KC // 8, 8, TQ), axis=0)
            return sm if m8 is None else jnp.maximum(m8, sm)

        def pv_chunk(h, c, s_ref, m, acc):
            s = s_ref[pl.ds(c * KC, KC), :]
            p = jnp.exp2(s - m).astype(bf16)
            hs = h * 32 if isinstance(h, int) else pl.multiple_of(h * 32, 32)
            v = vt_s[pl.ds(hs, 32), pl.ds(c * KC, KC)]
            o = jnp.dot(v, p, preferred_element_type=f32)
            return o if acc is None else acc + o

        def finish(u, acc):
            qt = u // H; h = u % H
            o = acc * pl.reciprocal(acc[DH:DH + 1, :], approx=False)
            if isinstance(u, int):
                ot_s[h * 32:(h + 1) * 32, qt * TQ:(qt + 1) * TQ] = o
            else:
                ot_s[pl.ds(pl.multiple_of(h * 32, 32), 32), pl.ds(pl.multiple_of(qt * TQ, TQ), TQ)] = o

        def step(u, m, m8, s_cur, s_nxt, n_left):
            h = u % H
            acc = None
            m_nxt = None
            qw1 = qweights(u + 1) if n_left >= 1 else None
            qw2 = qweights(u + 2) if (n_left >= 2 and SK > 0) else None
            for c in range(NC):
                cc = c + SK
                if cc < NC:
                    if qw1 is not None:
                        m8 = qk_chunk(qw1, cc, s_nxt, m8)
                        if cc == NC - 1:
                            m_nxt = jnp.max(m8, axis=0, keepdims=True)
                            m8 = None
                elif qw2 is not None:
                    m8 = qk_chunk(qw2, cc - NC, s_cur, m8)
                acc = pv_chunk(h, c, s_cur, m, acc)
            finish(u, acc)
            return m_nxt, m8

        qw = qweights(0)
        m8 = None
        for c in range(NC):
            m8 = qk_chunk(qw, c, sA, m8)
        m0 = jnp.max(m8, axis=0, keepdims=True)
        m8 = None
        if SK > 0:
            qw = qweights(1)
            for c in range(SK):
                m8 = qk_chunk(qw, c, sB, m8)
        cp_wo.wait()
        cp_w1.wait()
        cp_w2.wait()
        woT_s[...] = wo_s[...].T
        w1T_s[...] = w1_s[...].T
        b1c_s[...] = jnp.broadcast_to(b1_ref[...].astype(f32).reshape(1, F), (128, F)).T
        b2c_s[...] = jnp.broadcast_to(b2_ref[...].astype(f32).reshape(1, D), (128, D)).T

        def body(i, carry):
            if SK > 0:
                m, m8 = carry
            else:
                m, m8 = carry, None
            for r in range(UNR):
                u = i * UNR + r
                m, m8 = step(u, m, m8, sA if r % 2 == 0 else sB, sB if r % 2 == 0 else sA, 2)
            return (m, m8) if SK > 0 else m
        carry = lax.fori_loop(0, NU // UNR - 1, body, (m0, m8) if SK > 0 else m0)
        if SK > 0:
            m, m8 = carry
        else:
            m, m8 = carry, None
        for r in range(UNR):
            u = NU - UNR + r
            m, m8 = step(u, m, m8, sA if r % 2 == 0 else sB, sB if r % 2 == 0 else sA, UNR - 1 - r)

        def out_cp(t):
            c0 = pl.multiple_of(t * T3, T3)
            return pltpu.make_async_copy(y_s.at[:, pl.ds(c0, T3)], out_hbm.at[:, pl.ds(c0, T3)], out_sem.at[t])

        def p3(t, carry):
            c0 = pl.multiple_of(t * T3, T3)
            o = jnp.concatenate([ot_s[h * 32:h * 32 + DH, pl.ds(c0, T3)] for h in range(H)], axis=0).astype(bf16)
            hT = xt_s[:, pl.ds(c0, T3)].astype(f32) + jnp.dot(woT_s[...], o, preferred_element_type=f32)
            ln2 = _ln_T(hT).astype(bf16)
            a = jnp.dot(w1T_s[...], ln2, preferred_element_type=f32)
            a = a + jnp.concatenate([b1c_s[...]] * (T3 // 128), axis=1)
            a = jnp.maximum(a, 0.0)
            a = (a * a).astype(bf16)
            y = jnp.dot(w2T_s[...], a, preferred_element_type=f32)
            y = y + hT + jnp.concatenate([b2c_s[...]] * (T3 // 128), axis=1)
            y_s[:, pl.ds(c0, T3)] = y.astype(bf16)
            out_cp(t).start()
            return carry
        lax.fori_loop(0, N3, p3, 0)
        for t in range(N3):
            out_cp(t).wait()

    scratch = [
        pltpu.VMEM((D, S), bf16),
        pltpu.VMEM((D, 3 * D), bf16),
        pltpu.VMEM((D, D), bf16),
        pltpu.VMEM((D, F), bf16),
        pltpu.VMEM((D, F), bf16),
        pltpu.VMEM((3 * D, D), bf16),
        pltpu.VMEM((D, D), bf16),
        pltpu.VMEM((F, D), bf16),
        pltpu.VMEM((F, 128), f32),
        pltpu.VMEM((D, 128), f32),
        pltpu.VMEM((G, S, GW), bf16),
        pltpu.VMEM((D, S), bf16),
        pltpu.VMEM((H * 32, S), bf16),
        pltpu.VMEM((H * 32, S), f32),
        pltpu.VMEM((S, TQ), f32),
        pltpu.VMEM((S, TQ), f32),
        pltpu.VMEM((D, S), bf16),
        pltpu.SemaphoreType.DMA((6,)),
        pltpu.SemaphoreType.DMA((N3,)),
    ]
    return kern, scratch


def build(name="v2", **cfg):
    kern, scratch = make_kernel(**cfg)
    anyspec = pl.BlockSpec(memory_space=pl.ANY)
    vspec = pl.BlockSpec(memory_space=pltpu.VMEM)

    @jax.jit
    def fn(A_x, A_wqkv, A_wo, B_x, B_w1, B_b1, B_w2, B_b2):
        xt = A_x.reshape(S, D).T
        out = pl.pallas_call(
            kern,
            out_shape=jax.ShapeDtypeStruct((D, S), bf16),
            in_specs=[anyspec, anyspec, anyspec, anyspec, vspec, anyspec, vspec],
            out_specs=anyspec,
            scratch_shapes=scratch,
            compiler_params=pltpu.CompilerParams(vmem_limit_bytes=100 * 1024 * 1024),
            name=name,
        )(xt, A_wqkv, A_wo, B_w1, B_b1, B_w2.T, B_b2)
        return out.T.reshape(1, S, D)
    return fn


_FN = build(name="fused_block", UNR=8)


@jax.jit
def pallas_sequential_preLN__mha_block__dense_activation_squared_relu__prompt_kernel(
    A_x: jax.Array,
    A_wqkv: jax.Array,
    A_wo: jax.Array,
    B_x: jax.Array,
    B_w1: jax.Array,
    B_b1: jax.Array,
    B_w2: jax.Array,
    B_b2: jax.Array,
):
    return _FN(A_x, A_wqkv, A_wo, B_x, B_w1, B_b1, B_w2, B_b2)
```

```python
import functools
import math

import jax
import jax.numpy as jnp
from jax import lax
import jax.experimental.pallas as pl
import jax.experimental.pallas.tpu as pltpu

bf16 = jnp.bfloat16
f32 = jnp.float32
u32 = jnp.uint32

S = 2048
D = 448
H = 16
DH = 28
HP = 32
F = 1792
EPS = 1e-5
QSCALE = (DH ** -0.5) * math.log2(math.e)


def _sum0(x, nch):
    n, t = x.shape
    if nch == 0:
        return jnp.sum(x, axis=0, keepdims=True)
    parts = [x[i * 8:(i + 1) * 8] for i in range(n // 8)]
    accs = parts[:nch]
    for i in range(nch, len(parts)):
        accs[i % nch] = accs[i % nch] + parts[i]
    while len(accs) > 1:
        accs = [accs[i] + accs[i + 1] for i in range(0, len(accs), 2)]
    return jnp.sum(accs[0], axis=0, keepdims=True)


def _ln_T(x, nch):
    mu = _sum0(x, nch) * (1.0 / D)
    xc = x - mu
    var = _sum0(xc * xc, nch) * (1.0 / D)
    return (xc * lax.rsqrt(var + EPS)).astype(bf16)


class _NoScope:
    def __enter__(self):
        return self

    def __exit__(self, *a):
        return False


def make_kernel(T1=256, T3=256, SK=2, LAG=2, SCOPES=False, N1=0, N2=4,
                NOFF=128, GSTEP=3, EG=64, KBN=6, KB0=4, KB1=8, KGATE=True, RG=0, WP0=4, WPS=6, WGATE=False, HB=2, FR=64, FSKIP=4):
    TQ = 256
    KC = 256
    NQ = S // TQ
    NC = S // KC
    NH = TQ // 128
    N3 = S // T3
    NI = NQ * NC
    AHEAD = NC + SK + LAG
    RO = NOFF // NC
    MR = (S - NOFF) // NC
    assert MR % 16 == 0 and RO % 8 == 0
    KP1 = (HB + 1) * DH
    scope = jax.named_scope if SCOPES else (lambda n: _NoScope())

    def kern(xt_hbm, wqkv_hbm, wo_hbm, w1_hbm, b1_hbm, w2t_hbm, b2_hbm, out_hbm,
             k_s, qt_s, qf_s, vt_s, kb_s, ot_s, sA, sB, y_s,
             xt_s, wqkv_s, wo_s, w1_s, w2T_s, wqkvT_s, woT_s, w1T_s, b1c_s, b2c_s, ko_s,
             b1_s, b2_s, z_s, in_sem, out_sem):
        def colcp(src, dst, a, n, k):
            return pltpu.make_async_copy(src.at[:, pl.ds(a, n)], dst.at[:, pl.ds(a, n)], in_sem.at[k])
        cp_wa = colcp(wqkv_hbm, wqkv_s, 384, 512, 0)
        cp_x0 = colcp(xt_hbm, xt_s, 0, 2 * T1, 1)
        cp_wb = colcp(wqkv_hbm, wqkv_s, 896, 448, 2)
        cp_wc = colcp(wqkv_hbm, wqkv_s, 0, 384, 3)
        cp_x1 = colcp(xt_hbm, xt_s, 2 * T1, S - 2 * T1, 4)
        late = [
            pltpu.make_async_copy(w1_hbm, w1_s, in_sem.at[5]),
            pltpu.make_async_copy(wo_hbm, wo_s, in_sem.at[6]),
            pltpu.make_async_copy(w2t_hbm, w2T_s, in_sem.at[7]),
            pltpu.make_async_copy(b1_hbm, b1_s, in_sem.at[8]),
            pltpu.make_async_copy(b2_hbm, b2_s, in_sem.at[9]),
        ]
        for c in [cp_wa, cp_x0, cp_wb, cp_wc, cp_x1]:
            c.start()
        z_s[0] = 0

        ones_tail = (lax.broadcasted_iota(jnp.int32, (HP - DH, T1), 0) == 0).astype(f32)
        zero_tail = jnp.zeros((HP - DH, T1), f32)

        def ln1(t):
            return _ln_T(xt_s[:, pl.ds(t * T1, T1)].astype(f32), N1)

        def pk(t, xn):
            kk = jnp.dot(wqkvT_s[D:2 * D, :], xn, preferred_element_type=f32)
            for g in range(H // 2):
                h = 2 * g
                kt = jnp.concatenate([kk[h * DH:(h + 1) * DH], zero_tail,
                                      kk[(h + 1) * DH:(h + 2) * DH], zero_tail], axis=0).astype(bf16)
                k_s[g, pl.ds(t * T1 // 2, T1 // 2), :] = pltpu.bitcast(kt.T, u32)
            if t == 0 and NOFF:
                ko_s[0:D, :] = kk[:, 0:128]
                ko_s[D:512, :] = jnp.zeros((512 - D, 128), f32)

        def pv(t, xn):
            vv = jnp.dot(wqkvT_s[2 * D:3 * D, :], xn, preferred_element_type=f32)
            for h in range(H):
                v = jnp.concatenate([vv[h * DH:(h + 1) * DH], ones_tail], axis=0).astype(bf16)
                vt_s[h * 16:(h + 1) * 16, pl.ds(t * T1, T1)] = pltpu.bitcast(v, u32)

        def pq(t, xn):
            qq = jnp.dot(wqkvT_s[0:D, :], xn, preferred_element_type=f32) * QSCALE
            for h in range(H):
                q = jnp.concatenate([qq[h * DH:(h + 1) * DH], zero_tail], axis=0)
                qt_s[h * 16:(h + 1) * 16, pl.ds(t * T1, T1)] = pltpu.bitcast(q.astype(bf16), u32)
                if NOFF:
                    for j in range(T1 // 128):
                        qf_s[t * (T1 // 128) + j, h * HP:(h + 1) * HP, :] = q[:, j * 128:(j + 1) * 128]

        def kb_make(r, gate=None, never=None):
            row = ko_s[pl.ds(r, 8, stride=0), :]
            if gate is not None:
                row = jnp.where(never, gate, row)
            row16 = jnp.concatenate([row, row], axis=0).astype(bf16)
            full = jnp.concatenate([row16] * 8, axis=0)
            val = full.T.astype(f32)[0:NOFF]
            kb_s[r] = val
            return val[NOFF - 8:NOFF]

        kbn = [0]

        def kb_some(n):
            if NOFF:
                for r in range(kbn[0], min(KP1, kbn[0] + n)):
                    kb_make(r)
                kbn[0] = min(KP1, kbn[0] + n)

        with scope("w_B0"):
            cp_wa.wait()
        wqkvT_s[384:896, :] = wqkv_s[:, 384:896].T
        with scope("w_B1"):
            cp_x0.wait()
        xn0 = ln1(0)
        xn1 = ln1(1)
        pk(0, xn0)
        with scope("w_B2"):
            cp_wb.wait()
            cp_wc.wait()
        for c in late:
            c.start()
        wqkvT_s[896:1344, :] = wqkv_s[:, 896:1344].T
        wqkvT_s[0:384, :] = wqkv_s[:, 0:384].T
        pk(1, xn1)
        pv(0, xn0)
        pq(0, xn0)
        with scope("w_B3"):
            cp_x1.wait()
        xn = ln1(2)
        kb_some(KBN)
        pv(1, xn1)
        kb_some(KBN)
        pq(1, xn1)
        for t in range(2, S // T1):
            kb_some(KBN)
            pk(t, xn)
            xn_next = ln1(t + 1) if t + 1 < S // T1 else None
            kb_some(KBN)
            pv(t, xn)
            kb_some(KBN)
            pq(t, xn)
            xn = xn_next
        kb_some(D)

        def hrow(h, n):
            return h * n if isinstance(h, int) else pl.multiple_of(h * n, n)

        def sbuf(qt):
            return sA if qt % 2 == 0 else sB

        def qk_chunk(h, par, qt, c, never):
            if qt >= NQ:
                h, par, qt = h + 1, 1 - par, qt - NQ
            s_ref = sbuf(qt)
            qw = pltpu.bitcast(qt_s[pl.ds(hrow(h, 16), 16), pl.ds(qt * TQ, TQ)], bf16)
            r0 = NOFF + c * MR
            g = h // 2 if isinstance(h, int) else lax.shift_right_logical(h, 1)
            if par == 0:
                kc = pltpu.bitcast(k_s[g, pl.ds(r0 // 2, MR // 2), 0:HP], bf16)
            else:
                kc = pltpu.bitcast(k_s[g, pl.ds(r0 // 2, MR // 2), :], bf16)
                qw = jnp.concatenate([jnp.zeros((HP, TQ), bf16), qw], axis=0)
            s = jnp.dot(kc, qw, preferred_element_type=f32)
            s_ref[pl.ds(r0, MR), :] = s
            sm = jnp.max(s.reshape(MR // 8, 8, TQ), axis=0)
            if RO:
                halves = []
                for half in range(NH):
                    acc = None
                    for d in range(DH):
                        kb = kb_s[h * DH + d, pl.ds(c * RO, RO), :].reshape(RO // 8, 8, 128)
                        qd = qf_s[qt * NH + half, pl.ds(h * HP + d, 8, stride=0), :]
                        if GSTEP and d % GSTEP == 0:
                            tr = min(MR - 8, (d * MR // DH) // 8 * 8)
                            qd = jnp.where(never, s[tr:tr + 8, half * 128:(half + 1) * 128], qd)
                        t = kb * qd[None]
                        acc = t if acc is None else acc + t
                    halves.append(acc)
                so = jnp.concatenate(halves, axis=2)
                s_ref[pl.ds(c * RO, RO), :] = so.reshape(RO, TQ)
                sm = jnp.maximum(sm, jnp.max(so, axis=0))
            return s, sm

        def ex_chunk(qt, c, m, gate, never):
            s_ref = sbuf(qt)
            if gate is None or not EG:
                return jnp.exp2(s_ref[pl.ds(c * KC, KC), :] - m).astype(bf16)
            m8 = jnp.broadcast_to(m, (8, TQ))
            parts = []
            for g in range(KC // EG):
                tr = min(MR - 8, (g * EG * MR // KC) // 8 * 8)
                mg = jnp.where(never, gate[tr:tr + 8, :], m8)
                s = s_ref[pl.ds(c * KC + g * EG, EG), :].reshape(EG // 8, 8, TQ)
                parts.append((s - mg[None]).reshape(EG, TQ))
            return jnp.exp2(jnp.concatenate(parts, axis=0)).astype(bf16)

        def pv_chunk(h, c, p, acc):
            v = pltpu.bitcast(vt_s[pl.ds(hrow(h, 16), 16), pl.ds(c * KC, KC)], bf16)
            o = jnp.dot(v, p, preferred_element_type=f32)
            return o if acc is None else acc + o

        def finish(h, qt, acc):
            o = acc * pl.reciprocal(acc[DH:DH + 1, :], approx=False)
            ot_s[pl.ds(hrow(h, HP), HP), pl.ds(qt * TQ, TQ)] = o

        rgate = {}

        def run(h0, nh, m, m8, last, extra):
            never = z_s[0] > 0
            tot = nh * NI
            ms = {0: m}
            pend = [ex_chunk(0, j, m, None, never) for j in range(LAG)]
            acc = None
            for i in range(tot):
                j = i + AHEAD
                gate = None
                if not (last and j >= tot):
                    hh, jj = divmod(j, NI) if j < tot else (nh - 1, j - (nh - 1) * NI)
                    gate, sm = qk_chunk(h0 + hh, hh % 2, jj // NC, jj % NC, never)
                    m8 = sm if m8 is None else jnp.maximum(m8, sm)
                    if j % NC == NC - 1:
                        ms[j // NC] = jnp.max(m8, axis=0, keepdims=True)
                        m8 = None
                hi, ii = divmod(i, NI)
                extra(i, gate, never)
                e = i + LAG
                if e < tot:
                    g2 = gate
                    if not last and i in rgate:
                        top = g2[0:8, 0:128]
                        for tok in rgate[i]:
                            top = jnp.maximum(top, tok)
                        top = jnp.concatenate([top, g2[0:8, 128:]], axis=1)
                        g2 = jnp.concatenate([top, g2[8:]], axis=0)
                    pend.append(ex_chunk((e // NC) % NQ, e % NC, ms[e // NC], g2, never))
                acc = pv_chunk(h0 + hi, i % NC, pend.pop(0), acc)
                if i % NC == NC - 1:
                    finish(h0 + hi, ii // NC, acc)
                    acc = None
            return ms.get(nh * NQ), m8

        never0 = z_s[0] > 0
        m8 = None
        for j in range(AHEAD):
            _, sm = qk_chunk(0, 0, j // NC, j % NC, never0)
            m8 = sm if m8 is None else jnp.maximum(m8, sm)
            if j % NC == NC - 1:
                m0 = jnp.max(m8, axis=0, keepdims=True)
                m8 = None

        NIT = H // HB - 1

        KPER = HB * DH

        def body(it, carry):
            rgate.clear()
            def extra(i, gate, never):
                if NOFF:
                    for j in range(KPER):
                        if KB0 + j * (HB * NI - KB0 - KB1) // KPER == i:
                            tok = kb_make(it * KPER + KP1 + j, gate[0:8, 0:128] if KGATE else None, never)
                            if RG:
                                rgate.setdefault(i + RG, []).append(tok)
            return run(it * HB, HB, carry[0], carry[1], False, extra)
        with scope("attn_loop"):
            m, m8 = lax.fori_loop(0, NIT, body, (m0, m8))

        with scope("w_B4"):
            for c in late:
                c.wait()

        def out_cp(t):
            cs = pl.ds(t * T3, T3)
            return pltpu.make_async_copy(y_s.at[:, cs], out_hbm.at[:, cs], out_sem.at[t])

        def stage_a(t):
            cs = pl.ds(t * T3, T3)
            o = jnp.concatenate([ot_s[h * HP:h * HP + DH, cs] for h in range(H)], axis=0).astype(bf16)
            hT = xt_s[:, cs].astype(f32) + jnp.dot(woT_s[...], o, preferred_element_type=f32)
            return hT, _ln_T(hT, N2)

        def stage_w1(ln2, r0, r1):
            a = jnp.dot(w1T_s[r0:r1, :], ln2, preferred_element_type=f32)
            a = a + jnp.concatenate([b1c_s[r0:r1, :]] * (T3 // 128), axis=1)
            a = jnp.maximum(a, 0.0)
            return (a * a).astype(bf16)

        def stage_w2(t, a, hT):
            cs = pl.ds(t * T3, T3)
            y = jnp.dot(w2T_s[...], a, preferred_element_type=f32)
            y = y + hT + jnp.concatenate([b2c_s[...]] * (T3 // 128), axis=1)
            y_s[:, cs] = y.astype(bf16)
            out_cp(t).start()

        st = {"n": 0, "a": []}

        def gated(x, gate, never):
            if not WGATE:
                return x
            g = jnp.concatenate([gate[0:8, 0:128]] * 2, axis=0).astype(x.dtype)
            top = jnp.where(never, g, x[0:16, 0:128])
            if x.shape[1] > 128:
                top = jnp.concatenate([top, x[0:16, 128:]], axis=1)
            return jnp.concatenate([top, x[16:]], axis=0)

        def extra_last(i, gate, never):
            idle = gate is None
            if i >= WP0 and (i - WP0) % WPS == 0:
                j = (i - WP0) // WPS
                if j < 14:
                    w1T_s[j * 128:(j + 1) * 128, :] = gated(w1_s[:, j * 128:(j + 1) * 128], gate, never).T
                elif j == 14:
                    woT_s[0:256, :] = gated(wo_s[:, 0:256], gate, never).T
                elif j == 15:
                    woT_s[256:D, :] = gated(wo_s[:, 256:D], gate, never).T
                elif j == 16:
                    b1c_s[...] = jnp.broadcast_to(b1_s[...].astype(f32).reshape(1, F), (128, F)).T
                    b2c_s[...] = jnp.broadcast_to(b2_s[...].astype(f32).reshape(1, D), (128, D)).T
            if idle:
                n = st["n"]
                if n == 0:
                    st["A"] = stage_a(0)
                elif n >= FSKIP:
                    r0 = (n - FSKIP) * FR
                    st["a"].append(stage_w1(st["A"][1], r0, r0 + FR))
                st["n"] = n + 1

        run(H - HB, HB, m, m8, True, extra_last)

        hT, ln2 = st["A"]
        done = len(st["a"]) * FR
        for t in range(N3):
            if t == 0:
                a = jnp.concatenate(st["a"] + [stage_w1(ln2, done, F)], axis=0)
            else:
                a = stage_w1(ln2, 0, F)
            nxt = stage_a(t + 1) if t + 1 < N3 else None
            stage_w2(t, a, hT)
            if nxt is not None:
                hT, ln2 = nxt
        with scope("w_out"):
            for t in range(N3):
                out_cp(t).wait()

    nk = max(NOFF, 8)
    scratch = [
        pltpu.VMEM((H // 2, S // 2, 2 * HP), u32),
        pltpu.VMEM((H * 16, S), u32),
        pltpu.VMEM((S // 128, H * HP, 128), f32),
        pltpu.VMEM((H * 16, S), u32),
        pltpu.VMEM((D + DH, nk, 128), f32),
        pltpu.VMEM((H * HP, S), f32),
        pltpu.VMEM((S, TQ), f32),
        pltpu.VMEM((S, TQ), f32),
        pltpu.VMEM((D, S), bf16),
        pltpu.VMEM((D, S), bf16),
        pltpu.VMEM((D, 3 * D), bf16),
        pltpu.VMEM((D, D), bf16),
        pltpu.VMEM((D, F), bf16),
        pltpu.VMEM((D, F), bf16),
        pltpu.VMEM((3 * D, D), bf16),
        pltpu.VMEM((D, D), bf16),
        pltpu.VMEM((F, D), bf16),
        pltpu.VMEM((F, 128), f32),
        pltpu.VMEM((D, 128), f32),
        pltpu.VMEM((512, 128), f32),
        pltpu.VMEM((F,), bf16),
        pltpu.VMEM((D,), bf16),
        pltpu.SMEM((1,), jnp.int32),
        pltpu.SemaphoreType.DMA((10,)),
        pltpu.SemaphoreType.DMA((N3,)),
    ]
    return kern, scratch


def build(name="v8", **cfg):
    kern, scratch = make_kernel(**cfg)
    anyspec = pl.BlockSpec(memory_space=pl.ANY)

    @jax.jit
    def fn(A_x, A_wqkv, A_wo, B_x, B_w1, B_b1, B_w2, B_b2):
        xt = A_x.reshape(S, D).T
        out = pl.pallas_call(
            kern,
            out_shape=jax.ShapeDtypeStruct((D, S), bf16),
            in_specs=[anyspec] * 7,
            out_specs=anyspec,
            scratch_shapes=scratch,
            compiler_params=pltpu.CompilerParams(vmem_limit_bytes=100 * 1024 * 1024),
            name=name,
        )(xt, A_wqkv, A_wo, B_w1, B_b1, B_w2.T, B_b2)
        return out.T.reshape(1, S, D)
    return fn


_FN = build(name="fused_block", RG=4)


@jax.jit
def pallas_sequential_preLN__mha_block__dense_activation_squared_relu__prompt_kernel(
    A_x: jax.Array,
    A_wqkv: jax.Array,
    A_wo: jax.Array,
    B_x: jax.Array,
    B_w1: jax.Array,
    B_b1: jax.Array,
    B_w2: jax.Array,
    B_b2: jax.Array,
):
    return _FN(A_x, A_wqkv, A_wo, B_x, B_w1, B_b1, B_w2, B_b2)
```

```python
import functools
import math

import jax
import jax.numpy as jnp
from jax import lax
import jax.experimental.pallas as pl
import jax.experimental.pallas.tpu as pltpu

bf16 = jnp.bfloat16
f32 = jnp.float32
u32 = jnp.uint32

S = 2048
D = 448
H = 16
DH = 28
HP = 32
F = 1792
EPS = 1e-5
QSCALE = (DH ** -0.5) * math.log2(math.e)


def _sum0(x, nch):
    n, t = x.shape
    if nch == 0:
        return jnp.sum(x, axis=0, keepdims=True)
    parts = [x[i * 8:(i + 1) * 8] for i in range(n // 8)]
    accs = parts[:nch]
    for i in range(nch, len(parts)):
        accs[i % nch] = accs[i % nch] + parts[i]
    while len(accs) > 1:
        accs = [accs[i] + accs[i + 1] for i in range(0, len(accs), 2)]
    return jnp.sum(accs[0], axis=0, keepdims=True)


def _ln_T(x, nch):
    mu = _sum0(x, nch) * (1.0 / D)
    xc = x - mu
    var = _sum0(xc * xc, nch) * (1.0 / D)
    return (xc * lax.rsqrt(var + EPS)).astype(bf16)


class _NoScope:
    def __enter__(self):
        return self

    def __exit__(self, *a):
        return False


def make_kernel(T1=256, T3=256, SK=2, LAG=2, SCOPES=False, NV=4, VS=(4, 8, 8), N0=0, LSPAN=1.0, RGF=0, CH=True, XM=None, XR=None, N1=0, N2=4,
                NOFF=128, GSTEP=3, EG=64, KBN=6, KB0=4, KB1=8, KGATE=False, RG=4, WP0=4, WPS=6, WGATE=False, HB=2, FR=64, FSKIP=4):
    TQ = 256
    KC = 256
    NQ = S // TQ
    NC = S // KC
    NH = TQ // 128
    N3 = S // T3
    NI = NQ * NC
    AHEAD = NC + SK + LAG
    assert NOFF % 16 == 0
    g8 = NOFF // 8
    ROS = [8 * ((c + 1) * g8 // NC - c * g8 // NC) for c in range(NC)]
    g16 = (S - NOFF) // 16
    MRS = [16 * ((c + 1) * g16 // NC - c * g16 // NC) for c in range(NC)]
    if XM is not None:
        MRS = list(XM)
    if XR is not None:
        ROS = list(XR)
    assert sum(MRS) == S - NOFF and sum(ROS) == NOFF
    ROO = [sum(ROS[:c]) for c in range(NC)]
    MRO = [NOFF + sum(MRS[:c]) for c in range(NC)]
    NKT = (NOFF + 127) // 128
    KP1 = (HB + 1) * DH
    scope = jax.named_scope if SCOPES else (lambda n: _NoScope())

    def kern(xt_hbm, wqkv_hbm, wo_hbm, w1_hbm, b1_hbm, w2t_hbm, b2_hbm, out_hbm,
             k_s, qt_s, qf_s, vt_s, kb_s, ot_s, sA, sB, p_s, y_s,
             xt_s, wqkv_s, wo_s, w1_s, w2T_s, wqkvT_s, woT_s, w1T_s, b1c_s, b2c_s, ko_s,
             b1_s, b2_s, z_s, in_sem):
        def colcp(src, dst, a, n, k):
            return pltpu.make_async_copy(src.at[:, pl.ds(a, n)], dst.at[:, pl.ds(a, n)], in_sem.at[k])
        cp_wv1 = colcp(wqkv_hbm, wqkv_s, 896, 256, 0)
        cp_xa = colcp(xt_hbm, xt_s, 0, T1, 1)
        cp_wv2 = colcp(wqkv_hbm, wqkv_s, 1152, 192, 2)
        cp_xb = colcp(xt_hbm, xt_s, T1, T1, 2)
        cp_xc = colcp(xt_hbm, xt_s, 2 * T1, (NV - 2) * T1, 3)
        cp_wkq = colcp(wqkv_hbm, wqkv_s, 0, 896, 6)
        cp_x1 = colcp(xt_hbm, xt_s, NV * T1, S - NV * T1, 7)
        late = [
            pltpu.make_async_copy(w1_hbm, w1_s, in_sem.at[4]),
            pltpu.make_async_copy(wo_hbm, wo_s, in_sem.at[4]),
            pltpu.make_async_copy(w2t_hbm, w2T_s, in_sem.at[4]),
            pltpu.make_async_copy(b1_hbm, b1_s, in_sem.at[4]),
            pltpu.make_async_copy(b2_hbm, b2_s, in_sem.at[4]),
        ]
        for c in [cp_wv1, cp_xa, cp_wv2, cp_xb, cp_xc, cp_wkq, cp_x1]:
            c.start()
        z_s[0] = 0

        ones_tail = (lax.broadcasted_iota(jnp.int32, (HP - DH, T1), 0) == 0).astype(f32)
        zero_tail = jnp.zeros((HP - DH, T1), f32)

        def ln1(t):
            return _ln_T(xt_s[:, pl.ds(t * T1, T1)].astype(f32), N1)

        def pk(t, xn):
            kk = jnp.dot(wqkvT_s[D:2 * D, :], xn, preferred_element_type=f32)
            for g in range(H // 2):
                h = 2 * g
                kt = jnp.concatenate([kk[h * DH:(h + 1) * DH], zero_tail,
                                      kk[(h + 1) * DH:(h + 2) * DH], zero_tail], axis=0).astype(bf16)
                k_s[g, pl.ds(t * T1 // 2, T1 // 2), :] = pltpu.bitcast(kt.T, u32)
            if t == 0 and NOFF:
                for j in range(NKT):
                    ko_s[j, 0:D, :] = kk[:, j * 128:(j + 1) * 128]
                    ko_s[j, D:512, :] = jnp.zeros((512 - D, 128), f32)

        def pv(t, xn, ha=0, hb=H):
            vv = jnp.dot(wqkvT_s[2 * D + ha * DH:2 * D + hb * DH, :], xn, preferred_element_type=f32)
            for h in range(ha, hb):
                v = jnp.concatenate([vv[(h - ha) * DH:(h - ha + 1) * DH], ones_tail], axis=0).astype(bf16)
                vt_s[h * 16:(h + 1) * 16, pl.ds(t * T1, T1)] = pltpu.bitcast(v, u32)

        def pq(t, xn):
            qq = jnp.dot(wqkvT_s[0:D, :], xn, preferred_element_type=f32) * QSCALE
            for h in range(H):
                q = jnp.concatenate([qq[h * DH:(h + 1) * DH], zero_tail], axis=0)
                qt_s[h * 16:(h + 1) * 16, pl.ds(t * T1, T1)] = pltpu.bitcast(q.astype(bf16), u32)
                if NOFF:
                    for j in range(T1 // 128):
                        qf_s[t * (T1 // 128) + j, h * HP:(h + 1) * HP, :] = q[:, j * 128:(j + 1) * 128]

        def kb_make(r, gate=None, never=None):
            toks = []
            for j in range(NKT):
                row = ko_s[j, pl.ds(r, 8, stride=0), :]
                if gate is not None:
                    row = jnp.where(never, gate, row)
                n = min(128, NOFF - j * 128)
                row16 = jnp.concatenate([row, row], axis=0).astype(bf16)
                full = jnp.concatenate([row16] * 8, axis=0)
                val = full.T[0:n].astype(f32)
                kb_s[r, pl.ds(j * 128, n), :] = val
                toks.append(val[n - 8:n])
            return toks

        kbn = [0]

        def kb_some(n):
            if NOFF:
                for r in range(kbn[0], min(KP1, kbn[0] + n)):
                    kb_make(r)
                kbn[0] = min(KP1, kbn[0] + n)

        xns = {}
        with scope("w_B0"):
            cp_wv1.wait()
        wqkvT_s[896:1152, :] = wqkv_s[:, 896:1152].T
        with scope("w_B1"):
            cp_xa.wait()
        xns[0] = jnp.concatenate([_ln_T(xt_s[:, pl.ds(j * 128, 128)].astype(f32), N0) for j in range(T1 // 128)], axis=1)
        pv(0, xns[0], 0, VS[0])
        with scope("w_B2"):
            cp_wv2.wait()
            cp_xb.wait()
        wqkvT_s[1152:1344, :] = wqkv_s[:, 1152:1344].T
        xns[1] = ln1(1)
        pv(0, xns[0], VS[0], 8)
        pv(0, xns[0], 8, H)
        pv(1, xns[1], 0, VS[1])
        with scope("w_B3"):
            cp_xc.wait()
        xns[2] = ln1(2)
        pv(1, xns[1], VS[1], H)
        for t in range(2, NV - 1):
            xns[t + 1] = ln1(t + 1)
            pv(t, xns[t])
        pv(NV - 1, xns[NV - 1], 0, VS[2])
        with scope("w_B5"):
            cp_wkq.wait()
        wqkvT_s[384:896, :] = wqkv_s[:, 384:896].T
        wqkvT_s[0:384, :] = wqkv_s[:, 0:384].T
        pv(NV - 1, xns[NV - 1], VS[2], H)
        for t in range(NV):
            pk(t, xns[t])
            if t > 0:
                kb_some(KBN)
                pq(t - 1, xns[t - 1])
        with scope("w_B6"):
            cp_x1.wait()
        for c in late:
            c.start()
        xn = ln1(NV)
        kb_some(KBN)
        pq(NV - 1, xns[NV - 1])
        for t in range(NV, S // T1):
            kb_some(KBN)
            pk(t, xn)
            xn_next = ln1(t + 1) if t + 1 < S // T1 else None
            kb_some(KBN)
            pv(t, xn)
            kb_some(KBN)
            pq(t, xn)
            xn = xn_next
        kb_some(D)

        def hrow(h, n):
            return h * n if isinstance(h, int) else pl.multiple_of(h * n, n)

        def sbuf(qt):
            return sA if qt % 2 == 0 else sB

        def qk_chunk(h, par, qt, c, never, span=1.0):
            if qt >= NQ:
                h, par, qt = h + 1, 1 - par, qt - NQ
            s_ref = sbuf(qt)
            qw = pltpu.bitcast(qt_s[pl.ds(hrow(h, 16), 16), pl.ds(qt * TQ, TQ)], bf16)
            r0 = MRO[c]
            MR = MRS[c]
            RO = ROS[c]
            g = h // 2 if isinstance(h, int) else lax.shift_right_logical(h, 1)
            if par == 0:
                kc = pltpu.bitcast(k_s[g, pl.ds(r0 // 2, MR // 2), 0:HP], bf16)
            else:
                kc = pltpu.bitcast(k_s[g, pl.ds(r0 // 2, MR // 2), :], bf16)
                qw = jnp.concatenate([jnp.zeros((HP, TQ), bf16), qw], axis=0)
            s = jnp.dot(kc, qw, preferred_element_type=f32)
            s_ref[pl.ds(r0, MR), :] = s
            sm = jnp.max(s.reshape(MR // 8, 8, TQ), axis=0)
            if RO:
                halves = []
                for half in range(NH):
                    acc = None
                    for d in range(DH):
                        kb = kb_s[h * DH + d, pl.ds(ROO[c], RO), :].reshape(RO // 8, 8, 128)
                        qd = qf_s[qt * NH + half, pl.ds(h * HP + d, 8, stride=0), :]
                        if GSTEP and d % GSTEP == 0:
                            tr = min(MR - 8, int(d * MR * span / DH) // 8 * 8)
                            qd = jnp.where(never, s[tr:tr + 8, half * 128:(half + 1) * 128], qd)
                        t = kb * qd[None]
                        acc = t if acc is None else acc + t
                    halves.append(acc)
                so = jnp.concatenate(halves, axis=2)
                s_ref[pl.ds(ROO[c], RO), :] = so.reshape(RO, TQ)
                sm = jnp.maximum(sm, jnp.max(so, axis=0))
            return s, sm

        def ex_chunk(qt, c, m, gate, never):
            s_ref = sbuf(qt)
            if gate is None or not EG:
                return jnp.exp2(s_ref[pl.ds(c * KC, KC), :] - m).astype(bf16)
            m8 = jnp.broadcast_to(m, (8, TQ))
            MR = gate.shape[0]
            parts = []
            for g in range(KC // EG):
                tr = min(MR - 8, (g * EG * MR // KC) // 8 * 8)
                mg = jnp.where(never, gate[tr:tr + 8, :], m8)
                s = s_ref[pl.ds(c * KC + g * EG, EG), :].reshape(EG // 8, 8, TQ)
                parts.append((s - mg[None]).reshape(EG, TQ))
            return jnp.exp2(jnp.concatenate(parts, axis=0)).astype(bf16)

        def pv_chunk(h, c, p, acc):
            v = pltpu.bitcast(vt_s[pl.ds(hrow(h, 16), 16), pl.ds(c * KC, KC)], bf16)
            o = jnp.dot(v, p, preferred_element_type=f32)
            return o if acc is None else acc + o

        def finish(h, qt, acc):
            o = acc * pl.reciprocal(acc[DH:DH + 1, :], approx=False)
            ot_s[pl.ds(hrow(h, HP), HP), pl.ds(qt * TQ, TQ)] = o

        rgate = {}

        def run(h0, nh, m, m8, pend, last, extra):
            never = z_s[0] > 0
            tot = nh * NI
            rgate.clear()
            ms = {0: m}
            pend = [pltpu.bitcast(p_s[j], bf16) for j in range(LAG)]
            acc = None
            for i in range(tot):
                j = i + AHEAD
                gate = None
                if not (last and j >= tot):
                    hh, jj = divmod(j, NI) if j < tot else (nh - 1, j - (nh - 1) * NI)
                    gate, sm = qk_chunk(h0 + hh, hh % 2, jj // NC, jj % NC, never, LSPAN if i >= tot - 2 else 1.0)
                    m8 = sm if m8 is None else jnp.maximum(m8, sm)
                    if j % NC == NC - 1:
                        ms[j // NC] = jnp.max(m8, axis=0, keepdims=True)
                        m8 = None
                hi, ii = divmod(i, NI)
                extra(i, gate, never)
                e = i + LAG
                if e < tot or not last:
                    g2 = gate
                    if gate is not None and i in rgate:
                        top = g2[0:8, 0:128]
                        for tok in rgate[i]:
                            top = jnp.maximum(top, tok)
                        top = jnp.concatenate([top, g2[0:8, 128:]], axis=1)
                        g2 = jnp.concatenate([top, g2[8:]], axis=0)
                    pend.append(ex_chunk((e // NC) % NQ, e % NC, ms[e // NC], g2, never))
                acc = pv_chunk(h0 + hi, i % NC, pend.pop(0), acc)
                if i % NC == NC - 1:
                    finish(h0 + hi, ii // NC, acc)
                    if RGF:
                        rgate.setdefault(i + RGF, []).extend([acc[24:32, 0:128], acc[24:32, 128:256]])
                    if CH:
                        acc = jnp.concatenate([jnp.zeros((24, TQ), f32), jnp.where(never, acc[24:32], 0.0)], axis=0)
                    else:
                        acc = None
            if not last:
                for j in range(LAG):
                    p_s[j] = pltpu.bitcast(pend[j], u32)
            return ms.get(nh * NQ), m8

        never0 = z_s[0] > 0
        m8 = None
        for j in range(AHEAD):
            _, sm = qk_chunk(0, 0, j // NC, j % NC, never0)
            m8 = sm if m8 is None else jnp.maximum(m8, sm)
            if j % NC == NC - 1:
                m0 = jnp.max(m8, axis=0, keepdims=True)
                m8 = None

        for j in range(LAG):
            p_s[j] = pltpu.bitcast(ex_chunk(0, j, m0, None, never0), u32)
        NIT = H // HB - 1

        KPER = HB * DH

        def body(it, carry):
            def extra(i, gate, never):
                if NOFF:
                    for j in range(KPER):
                        if KB0 + j * (HB * NI - KB0 - KB1) // KPER == i:
                            tok = kb_make(it * KPER + KP1 + j, gate[0:8, 0:128] if KGATE else None, never)
                            if RG:
                                rgate.setdefault(i + RG, []).extend(tok)
            return run(it * HB, HB, carry[0], carry[1], None, False, extra)
        with scope("attn_loop"):
            m, m8 = lax.fori_loop(0, NIT, body, (m0, m8))

        with scope("w_B4"):
            for c in late:
                c.wait()

        def out_cp(t):
            cs = pl.ds(t * T3, T3)
            return pltpu.make_async_copy(y_s.at[:, cs], out_hbm.at[:, cs], in_sem.at[5])

        def stage_a(t):
            cs = pl.ds(t * T3, T3)
            o = jnp.concatenate([ot_s[h * HP:h * HP + DH, cs] for h in range(H)], axis=0).astype(bf16)
            hT = xt_s[:, cs].astype(f32) + jnp.dot(woT_s[...], o, preferred_element_type=f32)
            return hT, _ln_T(hT, N2)

        def stage_w1(ln2, r0, r1):
            a = jnp.dot(w1T_s[r0:r1, :], ln2, preferred_element_type=f32)
            a = a + jnp.concatenate([b1c_s[r0:r1, :]] * (T3 // 128), axis=1)
            a = jnp.maximum(a, 0.0)
            return (a * a).astype(bf16)

        def stage_w2(t, a, hT):
            cs = pl.ds(t * T3, T3)
            y = jnp.dot(w2T_s[...], a, preferred_element_type=f32)
            y = y + hT + jnp.concatenate([b2c_s[...]] * (T3 // 128), axis=1)
            y_s[:, cs] = y.astype(bf16)
            out_cp(t).start()

        st = {"n": 0, "a": []}

        def gated(x, gate, never):
            if not WGATE:
                return x
            g = jnp.concatenate([gate[0:8, 0:128]] * 2, axis=0).astype(x.dtype)
            top = jnp.where(never, g, x[0:16, 0:128])
            if x.shape[1] > 128:
                top = jnp.concatenate([top, x[0:16, 128:]], axis=1)
            return jnp.concatenate([top, x[16:]], axis=0)

        def extra_last(i, gate, never):
            idle = gate is None
            if i >= WP0 and (i - WP0) % WPS == 0:
                j = (i - WP0) // WPS
                if j < 14:
                    w1T_s[j * 128:(j + 1) * 128, :] = gated(w1_s[:, j * 128:(j + 1) * 128], gate, never).T
                elif j == 14:
                    woT_s[0:256, :] = gated(wo_s[:, 0:256], gate, never).T
                elif j == 15:
                    woT_s[256:D, :] = gated(wo_s[:, 256:D], gate, never).T
                elif j == 16:
                    b1c_s[...] = jnp.broadcast_to(b1_s[...].astype(f32).reshape(1, F), (128, F)).T
                    b2c_s[...] = jnp.broadcast_to(b2_s[...].astype(f32).reshape(1, D), (128, D)).T
            if idle:
                n = st["n"]
                if n == 0:
                    st["A"] = stage_a(0)
                elif n >= FSKIP:
                    r0 = (n - FSKIP) * FR
                    st["a"].append(stage_w1(st["A"][1], r0, r0 + FR))
                st["n"] = n + 1

        run(H - HB, HB, m, m8, None, True, extra_last)

        hT, ln2 = st["A"]
        done = len(st["a"]) * FR
        for t in range(N3):
            if t == 0:
                a = jnp.concatenate(st["a"] + [stage_w1(ln2, done, F)], axis=0)
            else:
                a = stage_w1(ln2, 0, F)
            nxt = stage_a(t + 1) if t + 1 < N3 else None
            stage_w2(t, a, hT)
            if nxt is not None:
                hT, ln2 = nxt
        with scope("w_out"):
            for t in range(N3):
                out_cp(t).wait()

    nk = max((NOFF + 31) // 32 * 32, 32)
    scratch = [
        pltpu.VMEM((H // 2, S // 2, 2 * HP), u32),
        pltpu.VMEM((H * 16, S), u32),
        pltpu.VMEM((S // 128, H * HP, 128), f32),
        pltpu.VMEM((H * 16, S), u32),
        pltpu.VMEM((D + DH, nk, 128), f32),
        pltpu.VMEM((H * HP, S), f32),
        pltpu.VMEM((S, TQ), f32),
        pltpu.VMEM((S, TQ), f32),
        pltpu.VMEM((LAG, KC // 2, TQ), u32),
        pltpu.VMEM((D, S), bf16),
        pltpu.VMEM((D, S), bf16),
        pltpu.VMEM((D, 3 * D), bf16),
        pltpu.VMEM((D, D), bf16),
        pltpu.VMEM((D, F), bf16),
        pltpu.VMEM((D, F), bf16),
        pltpu.VMEM((3 * D, D), bf16),
        pltpu.VMEM((D, D), bf16),
        pltpu.VMEM((F, D), bf16),
        pltpu.VMEM((F, 128), f32),
        pltpu.VMEM((D, 128), f32),
        pltpu.VMEM((max(NKT, 1), 512, 128), f32),
        pltpu.VMEM((F,), bf16),
        pltpu.VMEM((D,), bf16),
        pltpu.SMEM((1,), jnp.int32),
        pltpu.SemaphoreType.DMA((8,)),
    ]
    return kern, scratch


def build(name="v14", **cfg):
    kern, scratch = make_kernel(**cfg)
    anyspec = pl.BlockSpec(memory_space=pl.ANY)

    @jax.jit
    def fn(A_x, A_wqkv, A_wo, B_x, B_w1, B_b1, B_w2, B_b2):
        xt = A_x.reshape(S, D).T
        out = pl.pallas_call(
            kern,
            out_shape=jax.ShapeDtypeStruct((D, S), bf16),
            in_specs=[anyspec] * 7,
            out_specs=anyspec,
            scratch_shapes=scratch,
            compiler_params=pltpu.CompilerParams(vmem_limit_bytes=100 * 1024 * 1024),
            name=name,
        )(xt, A_wqkv, A_wo, B_w1, B_b1, B_w2.T, B_b2)
        return out.T.reshape(1, S, D)
    return fn


_FN = build(name="fused_block", EG=128)


@jax.jit
def pallas_sequential_preLN__mha_block__dense_activation_squared_relu__prompt_kernel(
    A_x: jax.Array,
    A_wqkv: jax.Array,
    A_wo: jax.Array,
    B_x: jax.Array,
    B_w1: jax.Array,
    B_b1: jax.Array,
    B_w2: jax.Array,
    B_b2: jax.Array,
):
    return _FN(A_x, A_wqkv, A_wo, B_x, B_w1, B_b1, B_w2, B_b2)
```

```python
import functools
import math

import jax
import jax.numpy as jnp
from jax import lax
import jax.experimental.pallas as pl
import jax.experimental.pallas.tpu as pltpu

bf16 = jnp.bfloat16
f32 = jnp.float32
u32 = jnp.uint32

S = 2048
D = 448
H = 16
DH = 28
HP = 32
F = 1792
EPS = 1e-5
QSCALE = (DH ** -0.5) * math.log2(math.e)


def _sum0(x, nch):
    n, t = x.shape
    if nch == 0:
        return jnp.sum(x, axis=0, keepdims=True)
    parts = [x[i * 8:(i + 1) * 8] for i in range(n // 8)]
    accs = parts[:nch]
    for i in range(nch, len(parts)):
        accs[i % nch] = accs[i % nch] + parts[i]
    while len(accs) > 1:
        accs = [accs[i] + accs[i + 1] for i in range(0, len(accs), 2)]
    return jnp.sum(accs[0], axis=0, keepdims=True)


def _ln_T(x, nch):
    mu = _sum0(x, nch) * (1.0 / D)
    xc = x - mu
    var = _sum0(xc * xc, nch) * (1.0 / D)
    return (xc * lax.rsqrt(var + EPS)).astype(bf16)


def _pk(x):
    return pltpu.bitcast(x, u32)


def _up(x):
    return pltpu.bitcast(x, bf16)


class _NoScope:
    def __enter__(self):
        return self

    def __exit__(self, *a):
        return False


def make_kernel(T1=256, T3=256, SK=2, LAG=2, SCOPES=False, NV=4, VS=(4, 8, 8), N0=0, LSPAN=1.0, RGF=0, CH=True, XM=None, XR=None, N1=0, N2=4,
                NOFF=128, GSTEP=3, EG=128, KBN=42, KREV=False, KF32=False, KB0=2, KB1=6, KGATE=False, RG=3, WP0=4, WPS=6, WGATE=False, HB=2, FA=2, FP=7, FSPAN=12, LCUT=(0, 224, 352, 448)):
    TQ = 256
    KC = 256
    NQ = S // TQ
    NC = S // KC
    NH = TQ // 128
    N3 = S // T3
    NI = NQ * NC
    AHEAD = NC + SK + LAG
    assert NOFF % 16 == 0
    g8 = NOFF // 8
    ROS = [8 * ((c + 1) * g8 // NC - c * g8 // NC) for c in range(NC)]
    g16 = (S - NOFF) // 16
    MRS = [16 * ((c + 1) * g16 // NC - c * g16 // NC) for c in range(NC)]
    if XM is not None:
        MRS = list(XM)
    if XR is not None:
        ROS = list(XR)
    assert sum(MRS) == S - NOFF and sum(ROS) == NOFF
    ROO = [sum(ROS[:c]) for c in range(NC)]
    MRO = [NOFF + sum(MRS[:c]) for c in range(NC)]
    NKT = (NOFF + 127) // 128
    KP1 = (HB + 1) * DH
    scope = jax.named_scope if SCOPES else (lambda n: _NoScope())

    def kern(xt_hbm, wqkv_hbm, wo_hbm, w1_hbm, b1_hbm, w2t_hbm, b2_hbm, out_hbm,
             k_s, qt_s, qf_s, vt_s, kb_s, ot_s, sA, sB, p_s, y_s,
             xt_s, wqkv_s, wo_s, w1_s, w2T_s, wqkvT_s, woT_s, w1T_s, w2p_s, b1c_s, b2c_s, ko_s,
             b1_s, b2_s, z_s, in_sem):
        def colcp(src, dst, a, n, k):
            return pltpu.make_async_copy(src.at[:, pl.ds(a, n)], dst.at[:, pl.ds(a, n)], in_sem.at[k])
        cp_wv1 = colcp(wqkv_hbm, wqkv_s, 896, 256, 0)
        cp_xa = colcp(xt_hbm, xt_s, 0, T1, 1)
        cp_wv2 = colcp(wqkv_hbm, wqkv_s, 1152, 192, 2)
        cp_xb = colcp(xt_hbm, xt_s, T1, T1, 2)
        cp_xc = colcp(xt_hbm, xt_s, 2 * T1, (NV - 2) * T1, 3)
        cp_wkq = colcp(wqkv_hbm, wqkv_s, 0, 896, 4)
        cp_x1 = colcp(xt_hbm, xt_s, NV * T1, S - NV * T1, 5)
        late = [
            pltpu.make_async_copy(w1_hbm, w1_s, in_sem.at[0]),
            pltpu.make_async_copy(wo_hbm, wo_s, in_sem.at[0]),
            pltpu.make_async_copy(w2t_hbm, w2T_s, in_sem.at[0]),
            pltpu.make_async_copy(b1_hbm, b1_s.at[pl.ds(0, F)], in_sem.at[0]),
            pltpu.make_async_copy(b2_hbm, b2_s, in_sem.at[0]),
        ]
        for c in [cp_wv1, cp_xa, cp_wv2, cp_xb, cp_xc, cp_wkq, cp_x1]:
            c.start()
        z_s[0] = 0

        ones_tail = (lax.broadcasted_iota(jnp.int32, (HP - DH, T1), 0) == 0).astype(f32)
        zero_tail = jnp.zeros((HP - DH, T1), f32)

        def ln1(t):
            return _ln_T(xt_s[:, pl.ds(t * T1, T1)].astype(f32), N1)

        def pk(t, xn):
            kk = jnp.dot(_up(wqkvT_s[D // 2:D, :]), xn, preferred_element_type=f32)
            for g in (range(H // 2) if t < S // T1 - 1 or not KREV else list(range(1, H // 2)) + [0]):
                h = 2 * g
                kt = jnp.concatenate([kk[h * DH:(h + 1) * DH], zero_tail,
                                      kk[(h + 1) * DH:(h + 2) * DH], zero_tail], axis=0).astype(bf16)
                k_s[g, pl.ds(t * T1 // 2, T1 // 2), :] = pltpu.bitcast(kt.T, u32)
            if t == 0 and NOFF:
                for j in range(NKT):
                    ko_s[j, 0:D, :] = kk[:, j * 128:(j + 1) * 128]
                    ko_s[j, D:512, :] = jnp.zeros((512 - D, 128), f32)

        def pv(t, xn, ha=0, hb=H):
            vv = jnp.dot(_up(wqkvT_s[D + ha * DH // 2:D + hb * DH // 2, :]), xn, preferred_element_type=f32)
            for h in range(ha, hb):
                v = jnp.concatenate([vv[(h - ha) * DH:(h - ha + 1) * DH], ones_tail], axis=0).astype(bf16)
                vt_s[h * 16:(h + 1) * 16, pl.ds(t * T1, T1)] = pltpu.bitcast(v, u32)
            return vv

        def pq(t, xn):
            qq = jnp.dot(_up(wqkvT_s[0:D // 2, :]), xn, preferred_element_type=f32) * QSCALE
            for h in range(H):
                q = jnp.concatenate([qq[h * DH:(h + 1) * DH], zero_tail], axis=0)
                qt_s[h * 16:(h + 1) * 16, pl.ds(t * T1, T1)] = pltpu.bitcast(q.astype(bf16), u32)
                if NOFF:
                    for j in range(T1 // 128):
                        qf_s[t * (T1 // 128) + j, h * HP:(h + 1) * HP, :] = q[:, j * 128:(j + 1) * 128]

        def kb_make(r, gate=None, never=None, wide=False):
            toks = []
            for j in range(NKT):
                row = ko_s[j, pl.ds(r, 8, stride=0), :]
                if gate is not None:
                    row = jnp.where(never, gate, row)
                n = min(128, NOFF - j * 128)
                if wide:
                    val = jnp.concatenate([row] * 16, axis=0).T[0:n]
                else:
                    row16 = jnp.concatenate([row, row], axis=0).astype(bf16)
                    full = jnp.concatenate([row16] * 8, axis=0)
                    val = full.T[0:n].astype(f32)
                kb_s[r, pl.ds(j * 128, n), :] = val
                toks.append(val[n - 8:n])
            return toks

        kbn = [0]

        def kb_some(n, src=None):
            if NOFF:
                rs = list(range(kbn[0], min(KP1, kbn[0] + n)))
                for k, r in enumerate(rs):
                    if src is None:
                        kb_make(r)
                    else:
                        pos = k * 2 * (D // 8) // len(rs)
                        half, tr = pos // (D // 8), pos % (D // 8) * 8
                        kb_make(r, src[tr:tr + 8, half * 128:(half + 1) * 128], z_s[0] > 0)
                kbn[0] = min(KP1, kbn[0] + n)

        xns = {}
        with scope("w_B0"):
            cp_wv1.wait()
        wqkvT_s[448:576, :] = _pk(wqkv_s[:, 896:1152].T)
        with scope("w_B1"):
            cp_xa.wait()
        xns[0] = jnp.concatenate([_ln_T(xt_s[:, pl.ds(j * 128, 128)].astype(f32), N0) for j in range(T1 // 128)], axis=1)
        pv(0, xns[0], 0, VS[0])
        with scope("w_B2"):
            cp_wv2.wait()
            cp_xb.wait()
        wqkvT_s[576:672, :] = _pk(wqkv_s[:, 1152:1344].T)
        xns[1] = ln1(1)
        pv(0, xns[0], VS[0], 8)
        pv(0, xns[0], 8, H)
        pv(1, xns[1], 0, VS[1])
        with scope("w_B3"):
            cp_xc.wait()
        xns[2] = ln1(2)
        pv(1, xns[1], VS[1], H)
        for t in range(2, NV - 1):
            xns[t + 1] = ln1(t + 1)
            pv(t, xns[t])
        pv(NV - 1, xns[NV - 1], 0, VS[2])
        with scope("w_B5"):
            cp_wkq.wait()
        wqkvT_s[192:448, :] = _pk(wqkv_s[:, 384:896].T)
        wqkvT_s[0:192, :] = _pk(wqkv_s[:, 0:384].T)
        pv(NV - 1, xns[NV - 1], VS[2], H)
        for t in range(NV):
            pk(t, xns[t])
            if t > 0:
                pq(t - 1, xns[t - 1])
        with scope("w_B6"):
            cp_x1.wait()
        for c in late:
            c.start()
        xn = ln1(NV)
        pq(NV - 1, xns[NV - 1])
        for t in range(NV, S // T1):
            pk(t, xn)
            xn_next = ln1(t + 1) if t + 1 < S // T1 else None
            vv = pv(t, xn)
            kb_some(KBN, vv)
            pq(t, xn)
            xn = xn_next
        kb_some(D)

        def hrow(h, n):
            return h * n if isinstance(h, int) else pl.multiple_of(h * n, n)

        def sbuf(qt):
            return sA if qt % 2 == 0 else sB

        def qk_chunk(h, par, qt, c, never, span=1.0):
            if qt >= NQ:
                h, par, qt = h + 1, 1 - par, qt - NQ
            s_ref = sbuf(qt)
            qw = pltpu.bitcast(qt_s[pl.ds(hrow(h, 16), 16), pl.ds(qt * TQ, TQ)], bf16)
            r0 = MRO[c]
            MR = MRS[c]
            RO = ROS[c]
            g = h // 2 if isinstance(h, int) else lax.shift_right_logical(h, 1)
            if par == 0:
                kc = pltpu.bitcast(k_s[g, pl.ds(r0 // 2, MR // 2), 0:HP], bf16)
            else:
                kc = pltpu.bitcast(k_s[g, pl.ds(r0 // 2, MR // 2), :], bf16)
                qw = jnp.concatenate([jnp.zeros((HP, TQ), bf16), qw], axis=0)
            s = jnp.dot(kc, qw, preferred_element_type=f32)
            s_ref[pl.ds(r0, MR), :] = s
            sm = jnp.max(s.reshape(MR // 8, 8, TQ), axis=0)
            if RO:
                halves = []
                for half in range(NH):
                    acc = None
                    for d in range(DH):
                        kb = kb_s[h * DH + d, pl.ds(ROO[c], RO), :].reshape(RO // 8, 8, 128)
                        qd = qf_s[qt * NH + half, pl.ds(h * HP + d, 8, stride=0), :]
                        if GSTEP and d % GSTEP == 0:
                            tr = min(MR - 8, int(d * MR * span / DH) // 8 * 8)
                            qd = jnp.where(never, s[tr:tr + 8, half * 128:(half + 1) * 128], qd)
                        t = kb * qd[None]
                        acc = t if acc is None else acc + t
                    halves.append(acc)
                so = jnp.concatenate(halves, axis=2)
                s_ref[pl.ds(ROO[c], RO), :] = so.reshape(RO, TQ)
                sm = jnp.maximum(sm, jnp.max(so, axis=0))
            return s, sm

        def ex_chunk(qt, c, m, gate, never):
            s_ref = sbuf(qt)
            if gate is None or not EG:
                return jnp.exp2(s_ref[pl.ds(c * KC, KC), :] - m).astype(bf16)
            m8 = jnp.broadcast_to(m, (8, TQ))
            MR = gate.shape[0]
            parts = []
            for g in range(KC // EG):
                tr = min(MR - 8, (g * EG * MR // KC) // 8 * 8)
                mg = jnp.where(never, gate[tr:tr + 8, :], m8)
                s = s_ref[pl.ds(c * KC + g * EG, EG), :].reshape(EG // 8, 8, TQ)
                parts.append((s - mg[None]).reshape(EG, TQ))
            return jnp.exp2(jnp.concatenate(parts, axis=0)).astype(bf16)

        def pv_chunk(h, c, p, acc):
            v = pltpu.bitcast(vt_s[pl.ds(hrow(h, 16), 16), pl.ds(c * KC, KC)], bf16)
            o = jnp.dot(v, p, preferred_element_type=f32)
            return o if acc is None else acc + o

        def finish(h, qt, acc):
            o = acc * pl.reciprocal(acc[DH:DH + 1, :], approx=False)
            ot_s[pl.ds(hrow(h, HP), HP), pl.ds(qt * TQ, TQ)] = o

        rgate = {}

        def run(h0, nh, m, m8, pend, last, extra):
            never = z_s[0] > 0
            tot = nh * NI
            rgate.clear()
            ms = {0: m}
            pend = [pltpu.bitcast(p_s[j], bf16) for j in range(LAG)]
            acc = None
            for i in range(tot):
                j = i + AHEAD
                gate = None
                if not (last and j >= tot):
                    hh, jj = divmod(j, NI) if j < tot else (nh - 1, j - (nh - 1) * NI)
                    gate, sm = qk_chunk(h0 + hh, hh % 2, jj // NC, jj % NC, never, LSPAN if i >= tot - 2 else 1.0)
                    m8 = sm if m8 is None else jnp.maximum(m8, sm)
                    if j % NC == NC - 1:
                        ms[j // NC] = jnp.max(m8, axis=0, keepdims=True)
                        m8 = None
                hi, ii = divmod(i, NI)
                extra(i, gate, never)
                e = i + LAG
                if e < tot or not last:
                    g2 = gate
                    if gate is not None and i in rgate:
                        top = g2[0:8, 0:128]
                        for tok in rgate[i]:
                            top = jnp.maximum(top, tok)
                        top = jnp.concatenate([top, g2[0:8, 128:]], axis=1)
                        g2 = jnp.concatenate([top, g2[8:]], axis=0)
                    pend.append(ex_chunk((e // NC) % NQ, e % NC, ms[e // NC], g2, never))
                acc = pv_chunk(h0 + hi, i % NC, pend.pop(0), acc)
                if i % NC == NC - 1:
                    finish(h0 + hi, ii // NC, acc)
                    if RGF:
                        rgate.setdefault(i + RGF, []).extend([acc[24:32, 0:128], acc[24:32, 128:256]])
                    if CH:
                        acc = jnp.concatenate([jnp.zeros((24, TQ), f32), jnp.where(never, acc[24:32], 0.0)], axis=0)
                    else:
                        acc = None
            if not last:
                for j in range(LAG):
                    p_s[j] = pltpu.bitcast(pend[j], u32)
            return ms.get(nh * NQ), m8

        never0 = z_s[0] > 0
        m8 = None
        for j in range(AHEAD):
            g0, sm = qk_chunk(0, 0, j // NC, j % NC, never0)
            m8 = sm if m8 is None else jnp.maximum(m8, sm)
            if j % NC == NC - 1:
                m0 = jnp.max(m8, axis=0, keepdims=True)
                m8 = None
            if j >= AHEAD - LAG:
                e = j - (AHEAD - LAG)
                p_s[e] = pltpu.bitcast(ex_chunk(0, e, m0, g0, never0), u32)

        NIT = H // HB - 1

        KPER = HB * DH

        def body(it, carry):
            def extra(i, gate, never):
                if NOFF:
                    for j in range(KPER):
                        if KB0 + j * (HB * NI - KB0 - KB1) // KPER == i:
                            tok = kb_make(it * KPER + KP1 + j, gate[0:8, 0:128] if KGATE else None, never, KF32)
                            if RG:
                                rgate.setdefault(i + RG, []).extend(tok)
            return run(it * HB, HB, carry[0], carry[1], None, False, extra)
        with scope("attn_loop"):
            m, m8 = lax.fori_loop(0, NIT, body, (m0, m8))

        with scope("w_B4"):
            for c in late:
                c.wait()

        def out_cp(t, r0=0, r1=D):
            cs = pl.ds(t * T3, T3)
            rs = pl.ds(r0, r1 - r0)
            return pltpu.make_async_copy(y_s.at[rs, cs], out_hbm.at[rs, cs], in_sem.at[1])

        outs = []

        def load_o(t):
            cs = pl.ds(t * T3, T3)
            return jnp.concatenate([ot_s[h * HP:h * HP + DH, cs] for h in range(H)], axis=0).astype(bf16)

        def h_rows(t, o, r0, r1):
            cs = pl.ds(t * T3, T3)
            return xt_s[r0:r1, cs].astype(f32) + jnp.dot(_up(woT_s[r0 // 2:r1 // 2, :]), o, preferred_element_type=f32)

        def stage_a(t):
            hT = h_rows(t, load_o(t), 0, D)
            return hT, _ln_T(hT, N2)

        def stage_w1(ln2, r0, r1):
            a = jnp.dot(_up(w1T_s[r0 // 2:r1 // 2, :]), ln2, preferred_element_type=f32)
            a = a + jnp.concatenate([b1c_s[r0:r1, :]] * (T3 // 128), axis=1)
            a = jnp.maximum(a, 0.0)
            return (a * a).astype(bf16)

        def stage_w2(t, a, hT):
            cs = pl.ds(t * T3, T3)
            y = jnp.dot(_up(w2p_s[...]), a, preferred_element_type=f32)
            y = y + hT + jnp.concatenate([b2c_s[...]] * (T3 // 128), axis=1)
            cuts = LCUT if t == N3 - 1 else (0, D)
            for r0, r1 in zip(cuts[:-1], cuts[1:]):
                y_s[r0:r1, cs] = y[r0:r1].astype(bf16)
                outs.append(out_cp(t, r0, r1))
                outs[-1].start()

        st = {"n": 0, "A": {}}
        pieces = [(tt, pi) for tt in range(FA) for pi in range(FP)]
        FPLAN = {}
        for k, pc in enumerate(pieces):
            FPLAN.setdefault(min(AHEAD - 1, k * FSPAN // len(pieces)), []).append(pc)

        def gated(x, gate, never):
            if not WGATE:
                return x
            g = jnp.concatenate([gate[0:8, 0:128]] * 2, axis=0).astype(x.dtype)
            top = jnp.where(never, g, x[0:16, 0:128])
            if x.shape[1] > 128:
                top = jnp.concatenate([top, x[0:16, 128:]], axis=1)
            return jnp.concatenate([top, x[16:]], axis=0)

        def extra_last(i, gate, never):
            idle = gate is None
            if i >= WP0 and (i - WP0) % WPS == 0:
                j = (i - WP0) // WPS
                if j < 14:
                    w1T_s[j * 64:(j + 1) * 64, :] = _pk(w1_s[:, j * 128:(j + 1) * 128].T)
                    w2p_s[:, j * 128:(j + 1) * 128] = _pk(w2T_s[:, j * 128:(j + 1) * 128])
                elif j == 14:
                    woT_s[0:128, :] = _pk(wo_s[:, 0:256].T)
                elif j == 15:
                    woT_s[128:D // 2, :] = _pk(wo_s[:, 256:D].T)
                elif j == 16:
                    b1c_s[...] = jnp.broadcast_to(b1_s[pl.ds(0, F)].astype(f32).reshape(1, F), (128, F)).T
                    b2c_s[...] = jnp.broadcast_to(b2_s[...].astype(f32).reshape(1, D), (128, D)).T
            if idle:
                n = st["n"]
                for (tt, pi) in FPLAN.get(n, []):
                    if pi == 0:
                        st["o"] = load_o(tt)
                        st["h"] = []
                    st["h"].append(h_rows(tt, st["o"], pi * D // FP, (pi + 1) * D // FP))
                    if pi == FP - 1:
                        hT = jnp.concatenate(st["h"], axis=0)
                        st["A"][tt] = (hT, _ln_T(hT, N2))
                st["n"] = n + 1

        run(H - HB, HB, m, m8, None, True, extra_last)

        A = st["A"]
        for t in range(N3):
            hT, ln2 = A.pop(t)
            a = stage_w1(ln2, 0, F)
            if t + 1 < N3 and t + 1 not in A:
                A[t + 1] = stage_a(t + 1)
            stage_w2(t, a, hT)
        with scope("w_out"):
            for c in outs:
                c.wait()

    nk = max((NOFF + 31) // 32 * 32, 32)
    scratch = [
        pltpu.VMEM((H // 2, S // 2, 2 * HP), u32),
        pltpu.VMEM((H * 16, S), u32),
        pltpu.VMEM((S // 128, H * HP, 128), f32),
        pltpu.VMEM((H * 16, S), u32),
        pltpu.VMEM((D + DH, nk, 128), f32),
        pltpu.VMEM((H * HP, S), f32),
        pltpu.VMEM((S, TQ), f32),
        pltpu.VMEM((S, TQ), f32),
        pltpu.VMEM((LAG, KC // 2, TQ), u32),
        pltpu.VMEM((D, S), bf16),
        pltpu.VMEM((D, S), bf16),
        pltpu.VMEM((D, 3 * D), bf16),
        pltpu.VMEM((D, D), bf16),
        pltpu.VMEM((D, F), bf16),
        pltpu.VMEM((D, F), bf16),
        pltpu.VMEM((3 * D // 2, D), u32),
        pltpu.VMEM((D // 2, D), u32),
        pltpu.VMEM((F // 2, D), u32),
        pltpu.VMEM((D // 2, F), u32),
        pltpu.VMEM((F, 128), f32),
        pltpu.VMEM((D, 128), f32),
        pltpu.VMEM((max(NKT, 1), 512, 128), f32),
        pltpu.VMEM((30 * 256,), bf16),
        pltpu.VMEM((D,), bf16),
        pltpu.SMEM((1,), jnp.int32),
        pltpu.SemaphoreType.DMA((6,)),
    ]
    return kern, scratch


def build(name="v17", **cfg):
    kern, scratch = make_kernel(**cfg)
    anyspec = pl.BlockSpec(memory_space=pl.ANY)

    @jax.jit
    def fn(A_x, A_wqkv, A_wo, B_x, B_w1, B_b1, B_w2, B_b2):
        xt = A_x.reshape(S, D).T
        out = pl.pallas_call(
            kern,
            out_shape=jax.ShapeDtypeStruct((D, S), bf16),
            in_specs=[anyspec] * 7,
            out_specs=anyspec,
            scratch_shapes=scratch,
            compiler_params=pltpu.CompilerParams(vmem_limit_bytes=100 * 1024 * 1024),
            name=name,
        )(xt, A_wqkv, A_wo, B_w1, B_b1, B_w2.T, B_b2)
        return out.T.reshape(1, S, D)
    return fn


_FN = build(name="fused_block")


@jax.jit
def pallas_sequential_preLN__mha_block__dense_activation_squared_relu__prompt_kernel(
    A_x: jax.Array,
    A_wqkv: jax.Array,
    A_wo: jax.Array,
    B_x: jax.Array,
    B_w1: jax.Array,
    B_b1: jax.Array,
    B_w2: jax.Array,
    B_b2: jax.Array,
):
    return _FN(A_x, A_wqkv, A_wo, B_x, B_w1, B_b1, B_w2, B_b2)
```

```python
import math

import jax
import jax.numpy as jnp
from jax import lax
import jax.experimental.pallas as pl
import jax.experimental.pallas.tpu as pltpu

bf16 = jnp.bfloat16
f32 = jnp.float32
u32 = jnp.uint32

S = 2048
D = 448
H = 16
DH = 28
HP = 32
F = 1792
EPS = 1e-5
QSCALE = (DH ** -0.5) * math.log2(math.e)

T = 256
NT = S // T
NI = NT * NT
NOFF = 128
RO = NOFF // NT
MR = (S - NOFF) // NT
HB = 2


def _pk(x):
    return pltpu.bitcast(x, u32)


def _up(x):
    return pltpu.bitcast(x, bf16)


def _sum0(x, nch):
    if nch == 1:
        return jnp.sum(x, axis=0, keepdims=True)
    parts = [x[i * 8:(i + 1) * 8] for i in range(x.shape[0] // 8)]
    accs = parts[:nch]
    for i in range(nch, len(parts)):
        accs[i % nch] = accs[i % nch] + parts[i]
    while len(accs) > 1:
        accs = [accs[i] + accs[i + 1] for i in range(0, len(accs), 2)]
    return jnp.sum(accs[0], axis=0, keepdims=True)


def _ln(x, nch):
    mu = _sum0(x, nch) * (1.0 / D)
    xc = x - mu
    var = _sum0(xc * xc, nch) * (1.0 / D)
    return (xc * lax.rsqrt(var + EPS)).astype(bf16)


def _dot(a, b):
    return jnp.dot(a, b, preferred_element_type=f32)


class _NoScope:
    def __enter__(self):
        return self

    def __exit__(self, *a):
        return False


def make_kernel(SCOPES=False, SK=2, LAG=2, GSTEP=3, EG=128, RG=3, KB0=2, KB1=6, KBN=42, NV=4,
                WP0=4, WPS=6, FP=7, LCUT=(0, 224, 352, 448), N0=4):
    AHEAD = NT + SK + LAG
    scope = jax.named_scope if SCOPES else (lambda n: _NoScope())

    def kern(xt_hbm, wqkv_hbm, wo_hbm, w1_hbm, b1_hbm, w2t_hbm, b2_hbm, out_hbm,
             k_s, qt_s, qf_s, vt_s, kb_s, ot_s, sA, sB, p_s, y_s,
             xt_s, wqkv_s, wo_s, w1_s, w2t_s, wqkvT_s, woT_s, w1T_s, w2p_s, b1c_s, b2c_s, ko_s,
             b1_s, b2_s, z_s, sem):
        def cols(t):
            return pl.ds(t * T, T)

        def colcp(src, dst, a, n, k):
            return pltpu.make_async_copy(src.at[:, pl.ds(a, n)], dst.at[:, pl.ds(a, n)], sem.at[k])

        cp_wv1 = colcp(wqkv_hbm, wqkv_s, 896, 256, 0)
        cp_xa = colcp(xt_hbm, xt_s, 0, T, 1)
        cp_wv2 = colcp(wqkv_hbm, wqkv_s, 1152, 192, 2)
        cp_xb = colcp(xt_hbm, xt_s, T, T, 2)
        cp_xc = colcp(xt_hbm, xt_s, 2 * T, (NV - 2) * T, 3)
        cp_wqk = colcp(wqkv_hbm, wqkv_s, 0, 896, 4)
        cp_xd = colcp(xt_hbm, xt_s, NV * T, S - NV * T, 5)
        late = [
            pltpu.make_async_copy(w1_hbm, w1_s, sem.at[0]),
            pltpu.make_async_copy(wo_hbm, wo_s, sem.at[0]),
            pltpu.make_async_copy(w2t_hbm, w2t_s, sem.at[0]),
            pltpu.make_async_copy(b1_hbm, b1_s.at[pl.ds(0, F)], sem.at[0]),
            pltpu.make_async_copy(b2_hbm, b2_s, sem.at[0]),
        ]
        for c in (cp_wv1, cp_xa, cp_wv2, cp_xb, cp_xc, cp_wqk, cp_xd):
            c.start()
        z_s[0] = 0

        ones_tail = (lax.broadcasted_iota(jnp.int32, (HP - DH, T), 0) == 0).astype(f32)
        zero_tail = jnp.zeros((HP - DH, T), f32)

        def wT(a, b):
            wqkvT_s[a // 2:b // 2, :] = _pk(wqkv_s[:, a:b].T)

        def ln1(t):
            return _ln(xt_s[:, cols(t)].astype(f32), 1)

        ktoks = []

        def proj_k(t, xn):
            kk = _dot(_up(wqkvT_s[D // 2:D, :]), xn)
            for g in range(H // 2):
                ka = jnp.concatenate([kk[2 * g * DH:(2 * g + 1) * DH], zero_tail], axis=0)
                kb = jnp.concatenate([kk[(2 * g + 1) * DH:(2 * g + 2) * DH], zero_tail], axis=0)
                if t == 0:
                    ko_s[2 * g] = ka[:, 0:NOFF]
                    ko_s[2 * g + 1] = kb[:, 0:NOFF]
                kt = _pk(jnp.concatenate([ka, kb], axis=0).astype(bf16).T)
                k_s[g, pl.ds(t * T // 2, T // 2), :] = kt
                if t == NT - 1 and g > 0:
                    tk = pltpu.bitcast(kt[T // 2 - 8:T // 2], f32)
                    ktoks.append(jnp.concatenate([tk] * 4, axis=1))
            if t == 0:
                ko_s[H] = jnp.zeros((HP, NOFF), f32)

        def proj_v(t, xn, ha=0, hb=H):
            vv = _dot(_up(wqkvT_s[D + ha * DH // 2:D + hb * DH // 2, :]), xn)
            for h in range(ha, hb):
                v = jnp.concatenate([vv[(h - ha) * DH:(h - ha + 1) * DH], ones_tail], axis=0)
                vt_s[h, :, cols(t)] = _pk(v.astype(bf16))
            return vv

        def proj_q(t, xn):
            qq = _dot(_up(wqkvT_s[0:D // 2, :]), xn) * QSCALE
            for h in range(H):
                q = jnp.concatenate([qq[h * DH:(h + 1) * DH], zero_tail], axis=0)
                qt_s[h, :, cols(t)] = _pk(q.astype(bf16))
                for j in range(T // 128):
                    qf_s[h, t * (T // 128) + j] = q[:, j * 128:(j + 1) * 128]

        def kb_make(h, d, gate=None, packed=False):
            row = jnp.broadcast_to(ko_s[h, d:d + 1, :], (8, NOFF))
            if gate is not None:
                row = jnp.where(z_s[0] > 0, gate, row)
            if packed:
                row = jnp.concatenate([row, row], axis=0).astype(bf16)
                val = jnp.concatenate([row] * 8, axis=0).T.astype(f32)
            else:
                val = jnp.concatenate([row] * 16, axis=0).T
            kb_s[h, d] = val.reshape(NOFF // 8, 8, 128)
            return val[NOFF - 8:NOFF]

        xn = {}
        with scope("w_B0"):
            cp_wv1.wait()
        wT(896, 1152)
        with scope("w_B1"):
            cp_xa.wait()
        xn[0] = jnp.concatenate([_ln(xt_s[:, j * 128:(j + 1) * 128].astype(f32), N0) for j in range(T // 128)], axis=1)
        proj_v(0, xn[0], 0, 4)
        with scope("w_B2"):
            cp_wv2.wait()
            cp_xb.wait()
        wT(1152, 1344)
        xn[1] = ln1(1)
        proj_v(0, xn[0], 4, 8)
        proj_v(0, xn[0], 8, H)
        proj_v(1, xn[1], 0, 8)
        with scope("w_B3"):
            cp_xc.wait()
        xn[2] = ln1(2)
        proj_v(1, xn[1], 8, H)
        for t in range(2, NV - 1):
            xn[t + 1] = ln1(t + 1)
            proj_v(t, xn[t])
        proj_v(NV - 1, xn[NV - 1], 0, 8)
        with scope("w_B5"):
            cp_wqk.wait()
        wT(384, 896)
        wT(0, 384)
        proj_v(NV - 1, xn[NV - 1], 8, H)
        for t in range(NV):
            proj_k(t, xn[t])
            if t > 0:
                proj_q(t - 1, xn[t - 1])
        with scope("w_B6"):
            cp_xd.wait()
        for c in late:
            c.start()
        xn[NV] = ln1(NV)
        proj_q(NV - 1, xn[NV - 1])
        todo = [(h, d) for h in range(HB + 1) for d in range(DH)]
        for t in range(NV, NT):
            proj_k(t, xn[t])
            if t + 1 < NT:
                xn[t + 1] = ln1(t + 1)
            vv = proj_v(t, xn[t])
            now, todo = todo[:KBN], todo[KBN:]
            for k, (h, d) in enumerate(now):
                half, tr = divmod(k * 2 * (D // 8) // len(now), D // 8)
                kb_make(h, d, vv[tr * 8:tr * 8 + 8, half * 128:(half + 1) * 128], packed=True)
            proj_q(t, xn[t])
        assert not todo

        def sbuf(qt):
            return sA if qt % 2 == 0 else sB

        def scores(h, g, odd, qt, c, never, toks=()):
            s_ref = sbuf(qt)
            qw = qt_s[h, :, cols(qt)]
            rows = pl.ds((NOFF + c * MR) // 2, MR // 2)
            if odd:
                kc = k_s[g, rows, :]
                qw = jnp.concatenate([jnp.zeros((HP // 2, T), u32), qw], axis=0)
            else:
                kc = k_s[g, rows, 0:HP]
            s = _dot(_up(kc), _up(qw))
            s_ref[pl.ds(NOFF + c * MR, MR), :] = s
            acc = None
            for d in range(DH):
                kb = kb_s[h, d, pl.ds(c * RO // 8, RO // 8)]
                qd = jnp.concatenate([jnp.broadcast_to(qf_s[h, qt * (T // 128) + j, d:d + 1, :], (8, 128))
                                      for j in range(T // 128)], axis=1)
                if d % GSTEP == 0:
                    tr = min(MR - 8, d * MR // DH // 8 * 8)
                    gate = s[tr:tr + 8]
                    if d == 0:
                        for tok in toks:
                            gate = jnp.maximum(gate, tok)
                    qd = jnp.where(never, gate, qd)
                t = jnp.concatenate([kb] * (T // 128), axis=2) * qd[None]
                acc = t if acc is None else acc + t
            s_ref[pl.ds(c * RO, RO), :] = acc.reshape(RO, T)
            return s, jnp.maximum(jnp.max(s.reshape(MR // 8, 8, T), axis=0), jnp.max(acc, axis=0))

        def probs(qt, c, m, s_now, never, toks=()):
            s_ref = sbuf(qt)
            if s_now is None:
                return jnp.exp2(s_ref[cols(c), :] - m).astype(bf16)
            m8 = jnp.broadcast_to(m, (8, T))
            parts = []
            for g in range(T // EG):
                tr = g * EG * MR // T // 8 * 8
                gate = s_now[tr:tr + 8]
                if g == 0 and toks:
                    left = gate[:, 0:128]
                    for tok in toks:
                        left = jnp.maximum(left, tok)
                    gate = jnp.concatenate([left, gate[:, 128:]], axis=1)
                s = s_ref[pl.ds(c * T + g * EG, EG), :].reshape(EG // 8, 8, T)
                parts.append((s - jnp.where(never, gate, m8)[None]).reshape(EG, T))
            return jnp.exp2(jnp.concatenate(parts, axis=0)).astype(bf16)

        def run(g0, m, m8, last, extra):
            never = z_s[0] > 0
            hs = [2 * g0 + k for k in range(HB + 1)]
            gs = [g0 + k for k in range(HB // 2 + 1)]
            tot = HB * NI
            ms = {0: m}
            toks = {}
            pend = [_up(p_s[j]) for j in range(LAG)]
            acc = None
            for i in range(tot):
                j = i + AHEAD
                s_now = None
                if j < tot or not last:
                    hh, jj = divmod(j, NI)
                    s_now, sm = scores(hs[hh], gs[hh // 2], hh % 2, jj // NT, jj % NT, never)
                    m8 = sm if m8 is None else jnp.maximum(m8, sm)
                    if j % NT == NT - 1:
                        ms[j // NT] = jnp.max(m8, axis=0, keepdims=True)
                        m8 = None
                tok = extra(i, s_now is None)
                if tok is not None:
                    toks.setdefault(i + RG, []).append(tok)
                e = i + LAG
                if e < tot or not last:
                    pend.append(probs(e // NT % NT, e % NT, ms[e // NT], s_now, never, toks.get(i, ())))
                hh, ii = divmod(i, NI)
                o = _dot(_up(vt_s[hs[hh], :, cols(i % NT)]), pend.pop(0))
                acc = o if acc is None else acc + o
                if i % NT == NT - 1:
                    ot_s[hs[hh], :, cols(ii // NT)] = acc * pl.reciprocal(acc[DH:DH + 1], approx=False)
                    acc = jnp.concatenate([jnp.zeros((HP - 8, T), f32),
                                           jnp.where(never, acc[HP - 8:HP], 0.0)], axis=0)
            if not last:
                for j in range(LAG):
                    p_s[j] = _pk(pend[j])
            return ms.get(HB * NT), m8

        never0 = z_s[0] > 0
        m8 = None
        for j in range(AHEAD):
            s_now, sm = scores(0, 0, 0, j // NT, j % NT, never0, ktoks if j == 0 else ())
            m8 = sm if m8 is None else jnp.maximum(m8, sm)
            if j % NT == NT - 1:
                m0 = jnp.max(m8, axis=0, keepdims=True)
                m8 = None
            if j >= AHEAD - LAG:
                p_s[j - (AHEAD - LAG)] = _pk(probs(0, j - (AHEAD - LAG), m0, s_now, never0))

        kb_at = {KB0 + j * (HB * NI - KB0 - KB1) // (HB * DH): j for j in range(HB * DH)}

        def body(it, carry):
            g0 = it * (HB // 2)
            nxt = [2 * g0 + HB + 1 + k for k in range(HB)]

            def extra(i, idle):
                if i in kb_at:
                    return kb_make(nxt[kb_at[i] // DH], kb_at[i] % DH)
            return run(g0, carry[0], carry[1], False, extra)

        with scope("attn_loop"):
            m, m8 = lax.fori_loop(0, H // HB - 1, body, (m0, m8))
        with scope("w_B4"):
            for c in late:
                c.wait()

        def load_o(t):
            return jnp.concatenate([ot_s[h, 0:DH, cols(t)] for h in range(H)], axis=0).astype(bf16)

        def h_rows(t, o, r0, r1):
            return xt_s[r0:r1, cols(t)].astype(f32) + _dot(_up(woT_s[r0 // 2:r1 // 2, :]), o)

        hid = {}
        st = {"n": 0}
        plan = {}
        for k in range(2 * FP):
            plan.setdefault(k * AHEAD // (2 * FP), []).append(divmod(k, FP))

        def extra_last(i, idle):
            j, r = divmod(i - WP0, WPS)
            if r == 0 and 0 <= j < 14:
                w1T_s[j * 64:(j + 1) * 64, :] = _pk(w1_s[:, j * 128:(j + 1) * 128].T)
                w2p_s[:, j * 128:(j + 1) * 128] = _pk(w2t_s[:, j * 128:(j + 1) * 128])
            elif r == 0 and j == 14:
                woT_s[0:128, :] = _pk(wo_s[:, 0:256].T)
            elif r == 0 and j == 15:
                woT_s[128:D // 2, :] = _pk(wo_s[:, 256:D].T)
            elif r == 0 and j == 16:
                b1c_s[...] = jnp.broadcast_to(b1_s[pl.ds(0, F)].astype(f32).reshape(1, F), (128, F)).T
                b2c_s[...] = jnp.broadcast_to(b2_s[...].astype(f32).reshape(1, D), (128, D)).T
            if idle:
                for t, pi in plan.get(st["n"], []):
                    if pi == 0:
                        st["o"] = load_o(t)
                        st["h"] = []
                    st["h"].append(h_rows(t, st["o"], pi * D // FP, (pi + 1) * D // FP))
                    if pi == FP - 1:
                        hT = jnp.concatenate(st["h"], axis=0)
                        hid[t] = (hT, _ln(hT, 4))
                st["n"] += 1

        run((H - HB) // 2, m, m8, True, extra_last)

        outs = []
        for t in range(NT):
            hT, ln2 = hid.pop(t)
            a = _dot(_up(w1T_s[...]), ln2) + jnp.concatenate([b1c_s[...]] * (T // 128), axis=1)
            a = jnp.maximum(a, 0.0)
            a = (a * a).astype(bf16)
            if t + 1 < NT and t + 1 not in hid:
                hn = h_rows(t + 1, load_o(t + 1), 0, D)
                hid[t + 1] = (hn, _ln(hn, 4))
            y = _dot(_up(w2p_s[...]), a) + hT + jnp.concatenate([b2c_s[...]] * (T // 128), axis=1)
            cuts = LCUT if t == NT - 1 else (0, D)
            for r0, r1 in zip(cuts[:-1], cuts[1:]):
                y_s[r0:r1, cols(t)] = y[r0:r1].astype(bf16)
                rs = pl.ds(r0, r1 - r0)
                outs.append(pltpu.make_async_copy(y_s.at[rs, cols(t)], out_hbm.at[rs, cols(t)], sem.at[1]))
                outs[-1].start()
        with scope("w_out"):
            for c in outs:
                c.wait()

    scratch = [
        pltpu.VMEM((H // 2, S // 2, 2 * HP), u32),
        pltpu.VMEM((H, HP // 2, S), u32),
        pltpu.VMEM((H, S // 128, HP, 128), f32),
        pltpu.VMEM((H, HP // 2, S), u32),
        pltpu.VMEM((H + 1, DH, NOFF // 8, 8, 128), f32),
        pltpu.VMEM((H, HP, S), f32),
        pltpu.VMEM((S, T), f32),
        pltpu.VMEM((S, T), f32),
        pltpu.VMEM((LAG, T // 2, T), u32),
        pltpu.VMEM((D, S), bf16),
        pltpu.VMEM((D, S), bf16),
        pltpu.VMEM((D, 3 * D), bf16),
        pltpu.VMEM((D, D), bf16),
        pltpu.VMEM((D, F), bf16),
        pltpu.VMEM((D, F), bf16),
        pltpu.VMEM((3 * D // 2, D), u32),
        pltpu.VMEM((D // 2, D), u32),
        pltpu.VMEM((F // 2, D), u32),
        pltpu.VMEM((D // 2, F), u32),
        pltpu.VMEM((F, 128), f32),
        pltpu.VMEM((D, 128), f32),
        pltpu.VMEM((H + 1, HP, NOFF), f32),
        pltpu.VMEM((30 * 256,), bf16),
        pltpu.VMEM((D,), bf16),
        pltpu.SMEM((1,), jnp.int32),
        pltpu.SemaphoreType.DMA((6,)),
    ]
    return kern, scratch


def build(name="v30", **cfg):
    kern, scratch = make_kernel(**cfg)
    anyspec = pl.BlockSpec(memory_space=pl.ANY)

    @jax.jit
    def fn(A_x, A_wqkv, A_wo, B_x, B_w1, B_b1, B_w2, B_b2):
        xt = A_x.reshape(S, D).T
        out = pl.pallas_call(
            kern,
            out_shape=jax.ShapeDtypeStruct((D, S), bf16),
            in_specs=[anyspec] * 7,
            out_specs=anyspec,
            scratch_shapes=scratch,
            compiler_params=pltpu.CompilerParams(vmem_limit_bytes=100 * 1024 * 1024),
            name=name,
        )(xt, A_wqkv, A_wo, B_w1, B_b1, B_w2.T, B_b2)
        return out.T.reshape(1, S, D)
    return fn


_FN = build(name="fused_block")


@jax.jit
def pallas_sequential_preLN__mha_block__dense_activation_squared_relu__prompt_kernel(
    A_x: jax.Array,
    A_wqkv: jax.Array,
    A_wo: jax.Array,
    B_x: jax.Array,
    B_w1: jax.Array,
    B_b1: jax.Array,
    B_w2: jax.Array,
    B_b2: jax.Array,
):
    return _FN(A_x, A_wqkv, A_wo, B_x, B_w1, B_b1, B_w2, B_b2)
```

```python
import math

import jax
import jax.numpy as jnp
from jax import lax
import jax.experimental.pallas as pl
import jax.experimental.pallas.tpu as pltpu

bf16 = jnp.bfloat16
f32 = jnp.float32
u32 = jnp.uint32

S = 2048
D = 448
H = 16
DH = 28
HP = 32
F = 1792
EPS = 1e-5
QSCALE = (DH ** -0.5) * math.log2(math.e)

T = 256
NT = S // T
NI = NT * NT
NOFF = 128
RO = NOFF // NT
MR = (S - NOFF) // NT
DA = D + 16
HB = 2


def _pk(x):
    return pltpu.bitcast(x, u32)


def _up(x):
    return pltpu.bitcast(x, bf16)


def _sum0(x, nch):
    if nch == 1:
        return jnp.sum(x, axis=0, keepdims=True)
    parts = [x[i * 8:(i + 1) * 8] for i in range(x.shape[0] // 8)]
    accs = parts[:nch]
    for i in range(nch, len(parts)):
        accs[i % nch] = accs[i % nch] + parts[i]
    while len(accs) > 1:
        accs = [accs[i] + accs[i + 1] for i in range(0, len(accs), 2)]
    return jnp.sum(accs[0], axis=0, keepdims=True)


def _ln(x, nch, extra=None):
    mu = _sum0(x, nch) * (1.0 / D)
    xc = x - mu
    r = lax.rsqrt(_sum0(xc * xc, nch) * (1.0 / D) + EPS)
    y = xc * r
    if extra is not None:
        y = jnp.concatenate([y, extra], axis=0)
    return y.astype(bf16)


def _dot(a, b):
    return jnp.dot(a, b, preferred_element_type=f32)


class _NoScope:
    def __enter__(self):
        return self

    def __exit__(self, *a):
        return False


def make_kernel(SCOPES=False, SK=2, LAG=2, GSTEP=3, EG=128, RG=3, KB0=3, KB1=13, WTOK=1, KBN=42, NV=4,
                WP0=3, WPS=5, FP=7, LCUT=(0, 224, 352, 448), N0=4, N2=2, ROH=(64, 80), BR=32, G2=3, KB2=4, FIRST=5, PG=True, QT=False, QS=2, P0=28, A0=(24, 25), LG=32, KV=1, KN=4, L0=None):
    NOFF2 = max(ROH) * NT
    NK2 = NOFF2 // 128
    jobs2 = [(hh, r, j) for r in range(4) for hh in range(2) for j in range(ROH[hh] * NT // 128)]
    AHEAD = NT + SK + LAG
    scope = jax.named_scope if SCOPES else (lambda n: _NoScope())

    def kern(xt_hbm, wqkv_hbm, wo_hbm, w1_hbm, b1_hbm, w2t_hbm, b2_hbm, out_hbm,
             k_s, qt_s, qf_s, vt_s, kb_s, kb2_s, ot_s, sA, sB, p_s, y_s,
             xt_s, wqkv_s, wo_s, w1_s, w2t_s, wqkvT_s, woT_s, w1T_s, w2p_s, b2c_s, ko_s, ko2_s,
             b1_s, b2_s, z_s, sem):
        def cols(t):
            return pl.ds(t * T, T)

        def colcp(src, dst, a, n, k):
            return pltpu.make_async_copy(src.at[:, pl.ds(a, n)], dst.at[:, pl.ds(a, n)], sem.at[k])

        cp_wv1 = colcp(wqkv_hbm, wqkv_s, 896, 256, 0)
        cp_xa = colcp(xt_hbm, xt_s, 0, T, 1)
        cp_wv2 = colcp(wqkv_hbm, wqkv_s, 1152, 192, 2)
        cp_xb = colcp(xt_hbm, xt_s, T, T, 2)
        cp_xc = colcp(xt_hbm, xt_s, 2 * T, (NV - 2) * T, 3)
        cp_wqk = colcp(wqkv_hbm, wqkv_s, 0, 896, 4)
        cp_xd = colcp(xt_hbm, xt_s, NV * T, S - NV * T, 5)
        late = [
            pltpu.make_async_copy(w1_hbm, w1_s.at[pl.ds(0, D)], sem.at[0]),
            pltpu.make_async_copy(wo_hbm, wo_s, sem.at[0]),
            pltpu.make_async_copy(w2t_hbm, w2t_s, sem.at[0]),
            pltpu.make_async_copy(b1_hbm, b1_s.at[pl.ds(0, F)], sem.at[0]),
            pltpu.make_async_copy(b2_hbm, b2_s, sem.at[0]),
        ]
        for c in (cp_wv1, cp_xa, cp_wv2, cp_xb, cp_xc, cp_wqk, cp_xd):
            c.start()
        z_s[0] = 0

        ones_tail = (lax.broadcasted_iota(jnp.int32, (HP - DH, T), 0) == 0).astype(f32)
        zero_tail = jnp.zeros((HP - DH, T), f32)

        def wT(a, b):
            wqkvT_s[a // 2:b // 2, :] = _pk(wqkv_s[:, a:b].T)

        def ln1(t):
            return _ln(xt_s[:, cols(t)].astype(f32), 1)

        ktoks = []

        def proj_k(t, xn):
            kk = _dot(_up(wqkvT_s[D // 2:D, :]), xn)
            for g in range(H // 2):
                ka = jnp.concatenate([kk[2 * g * DH:(2 * g + 1) * DH], zero_tail], axis=0)
                kb = jnp.concatenate([kk[(2 * g + 1) * DH:(2 * g + 2) * DH], zero_tail], axis=0)
                if t == 0:
                    ko_s[2 * g] = ka[:, 0:NOFF]
                    ko_s[2 * g + 1] = kb[:, 0:NOFF]
                kt = _pk(jnp.concatenate([ka, kb], axis=0).astype(bf16).T)
                k_s[g, pl.ds(t * T // 2, T // 2), :] = kt
                if t == NT - 1 and g > 0:
                    tk = pltpu.bitcast(kt[T // 2 - 8:T // 2], f32)
                    ktoks.append(jnp.concatenate([tk] * 4, axis=1))
            if t == 0:
                ko_s[H] = jnp.zeros((HP, NOFF), f32)
            for j in range(T // 128):
                if t * (T // 128) + j < NK2:
                    ko2_s[t * (T // 128) + j] = kk[D - 64:D, j * 128:(j + 1) * 128]

        def proj_v(t, xn, ha=0, hb=H):
            vv = _dot(_up(wqkvT_s[D + ha * DH // 2:D + hb * DH // 2, :]), xn)
            for h in range(ha, hb):
                v = jnp.concatenate([vv[(h - ha) * DH:(h - ha + 1) * DH], ones_tail], axis=0)
                vt_s[h, :, cols(t)] = _pk(v.astype(bf16))
            return vv

        def proj_q(t, xn):
            qq = _dot(_up(wqkvT_s[0:D // 2, :]), xn) * QSCALE
            for h in range(H):
                q = jnp.concatenate([qq[h * DH:(h + 1) * DH], zero_tail], axis=0)
                qt_s[h, :, cols(t)] = _pk(q.astype(bf16))
                for j in range(T // 128):
                    qf_s[h, t * (T // 128) + j] = q[:, j * 128:(j + 1) * 128]

        def kb_make(h, d, gate=None, packed=False):
            row = jnp.broadcast_to(ko_s[h, d:d + 1, :], (8, NOFF))
            if gate is not None:
                row = jnp.where(z_s[0] > 0, gate, row)
            if packed:
                row = jnp.concatenate([row, row], axis=0).astype(bf16)
                val = jnp.concatenate([row] * 8, axis=0).T.astype(f32)
            else:
                val = jnp.concatenate([row] * 16, axis=0).T
            kb_s[h, d] = val.reshape(NOFF // 8, 8, 128)
            return val[NOFF - 8:NOFF]

        def kb2_make(r, j):
            row = jnp.broadcast_to(ko2_s[j, pl.ds(64 - HB * DH + r, 1), :], (8, 128))
            val = jnp.concatenate([row] * 16, axis=0).T
            kb2_s[r, pl.ds(j * 16, 16)] = val.reshape(16, 8, 128)
            return val[120:128]

        xn = {}
        with scope("w_B0"):
            cp_wv1.wait()
        wT(896, 1152)
        with scope("w_B1"):
            cp_xa.wait()
        xn[0] = jnp.concatenate([_ln(xt_s[:, j * 128:(j + 1) * 128].astype(f32), N0) for j in range(T // 128)], axis=1)
        proj_v(0, xn[0], 0, 4)
        with scope("w_B2"):
            cp_wv2.wait()
            cp_xb.wait()
        wT(1152, 1344)
        xn[1] = ln1(1)
        proj_v(0, xn[0], 4, 8)
        proj_v(0, xn[0], 8, H)
        proj_v(1, xn[1], 0, 8)
        with scope("w_B3"):
            cp_xc.wait()
        xn[2] = ln1(2)
        proj_v(1, xn[1], 8, H)
        for t in range(2, NV - 1):
            xn[t + 1] = ln1(t + 1)
            proj_v(t, xn[t])
        proj_v(NV - 1, xn[NV - 1], 0, 8)
        with scope("w_B5"):
            cp_wqk.wait()
        wT(384, 896)
        wT(0, 384)
        proj_v(NV - 1, xn[NV - 1], 8, H)
        for t in range(NV):
            proj_k(t, xn[t])
            if t > 0:
                proj_q(t - 1, xn[t - 1])
        for c in late:
            c.start()
        with scope("w_B6"):
            cp_xd.wait()
        xn[NV] = ln1(NV)
        proj_q(NV - 1, xn[NV - 1])
        todo = [(h, d) for h in range(HB + 1) for d in range(DH)]
        for t in range(NV, NT):
            proj_k(t, xn[t])
            if t + 1 < NT:
                xn[t + 1] = ln1(t + 1)
            vv = proj_v(t, xn[t])
            now, todo = todo[:KBN], todo[KBN:]
            for k, (h, d) in enumerate(now):
                half, tr = divmod(k * 2 * (D // 8) // len(now), D // 8)
                kb_make(h, d, vv[tr * 8:tr * 8 + 8, half * 128:(half + 1) * 128], packed=True)
            proj_q(t, xn[t])
        assert not todo

        def sbuf(qt):
            return sA if qt % 2 == 0 else sB

        def scores(h, g, odd, qt, c, never, toks=(), buf=None):
            s_ref = sbuf(qt if buf is None else buf)
            qw = qt_s[h, :, cols(qt)]
            rows = pl.ds((NOFF + c * MR) // 2, MR // 2)
            if odd:
                kc = k_s[g, rows, :]
                qw = jnp.concatenate([jnp.zeros((HP // 2, T), u32), qw], axis=0)
            else:
                kc = k_s[g, rows, 0:HP]
            s = _dot(_up(kc), _up(qw))
            s_ref[pl.ds(NOFF + c * MR, MR), :] = s
            acc = None
            for d in range(DH):
                kb = kb_s[h, d, pl.ds(c * RO // 8, RO // 8)]
                qd = jnp.concatenate([jnp.broadcast_to(qf_s[h, qt * (T // 128) + j, d:d + 1, :], (8, 128))
                                      for j in range(T // 128)], axis=1)
                if d % GSTEP == 0:
                    tr = min(MR - 8, d * MR // DH // 8 * 8)
                    gate = s[tr:tr + 8]
                    if d == 0:
                        for tok in toks:
                            gate = jnp.maximum(gate, tok)
                    qd = jnp.where(never, gate, qd)
                t = jnp.concatenate([kb] * (T // 128), axis=2) * qd[None]
                acc = t if acc is None else acc + t
            s_ref[pl.ds(c * RO, RO), :] = acc.reshape(RO, T)
            return s, jnp.maximum(jnp.max(s.reshape(MR // 8, 8, T), axis=0), jnp.max(acc, axis=0))

        def probs(qt, c, m, s_now, never, toks=()):
            s_ref = sbuf(qt)
            if s_now is None:
                return jnp.exp2(s_ref[cols(c), :] - m).astype(bf16)
            m8 = jnp.broadcast_to(m, (8, T))
            parts = []
            for g in range(T // EG):
                tr = g * EG * MR // T // 8 * 8
                gate = s_now[tr:tr + 8]
                if g == 0 and toks:
                    left = gate[:, 0:128]
                    for tok in toks:
                        left = jnp.maximum(left, tok)
                    gate = jnp.concatenate([left, gate[:, 128:]], axis=1)
                s = s_ref[pl.ds(c * T + g * EG, EG), :].reshape(EG // 8, 8, T)
                parts.append((s - jnp.where(never, gate, m8)[None]).reshape(EG, T))
            return jnp.exp2(jnp.concatenate(parts, axis=0)).astype(bf16)

        def run(g0, m, m8, last, extra):
            never = z_s[0] > 0
            hs = [2 * g0 + k for k in range(HB + 1)]
            gs = [g0 + k for k in range(HB // 2 + 1)]
            tot = HB * NI
            ms = {0: m}
            toks = {}
            pend = [_up(p_s[j]) for j in range(LAG)]
            acc = None
            for i in range(tot):
                j = i + AHEAD
                s_now = None
                if j < tot or not last:
                    hh, jj = divmod(j, NI)
                    s_now, sm = scores(hs[hh], gs[hh // 2], hh % 2, jj // NT, jj % NT, never)
                    m8 = sm if m8 is None else jnp.maximum(m8, sm)
                    if j % NT == NT - 1:
                        ms[j // NT] = jnp.max(m8, axis=0, keepdims=True)
                        m8 = None
                tok = extra(i, s_now is None)
                if tok is not None:
                    toks.setdefault(i + RG, []).append(tok)
                e = i + LAG
                if e < tot or not last:
                    pend.append(probs(e // NT % NT, e % NT, ms[e // NT], s_now, never, toks.get(i, ())))
                hh, ii = divmod(i, NI)
                o = _dot(_up(vt_s[hs[hh], :, cols(i % NT)]), pend.pop(0))
                acc = o if acc is None else acc + o
                if i % NT == NT - 1:
                    ot_s[hs[hh], :, cols(ii // NT)] = _pk((acc * pl.reciprocal(acc[DH:DH + 1], approx=False)).astype(bf16))
                    acc = jnp.concatenate([jnp.zeros((HP - 8, T), f32),
                                           jnp.where(never, acc[HP - 8:HP], 0.0)], axis=0)
            if not last:
                for j in range(LAG):
                    p_s[j] = _pk(pend[j])
            return ms.get(HB * NT), m8

        never0 = z_s[0] > 0
        m8 = None
        for j in range(AHEAD):
            s_now, sm = scores(0, 0, 0, j // NT, j % NT, never0, ktoks if j == 0 else ())
            m8 = sm if m8 is None else jnp.maximum(m8, sm)
            if j % NT == NT - 1:
                m0 = jnp.max(m8, axis=0, keepdims=True)
                m8 = None
            if j >= AHEAD - LAG:
                p_s[j - (AHEAD - LAG)] = _pk(probs(0, j - (AHEAD - LAG), m0, s_now, never0))

        kb_at = {KB0 + j * (HB * NI - KB0 - KB1) // (HB * DH): j for j in range(HB * DH)}

        def body(it, carry):
            g0 = it * (HB // 2)
            nxt = [2 * g0 + HB + 1 + k for k in range(HB)]

            def extra(i, idle):
                if i in kb_at:
                    return kb_make(nxt[kb_at[i] // DH], kb_at[i] % DH)
                k = (i - KB2) // 2
                if 0 <= k < len(jobs2) and (i - KB2) % 2 == 0:
                    hh, r, j = jobs2[k]
                    return kb2_make(it * 4 + hh * DH + r, j)
            return run(g0, carry[0], carry[1], False, extra)

        with scope("attn_loop"):
            m, m8 = lax.fori_loop(0, H // HB - 1, body, (m0, m8))
        with scope("w_B4"):
            for c in late:
                c.wait()
        first_row = lax.broadcasted_iota(jnp.int32, (16, F), 0) == 0
        b1 = jnp.broadcast_to(b1_s[pl.ds(0, F)].astype(f32).reshape(1, F), (16, F))
        w1_s[D:DA, :] = jnp.where(first_row, b1, 0.0).astype(bf16)
        for j in range(F // 128):
            w1T_s[j * 64:(j + 1) * 64, :] = _pk(w1_s[0:DA, j * 128:(j + 1) * 128].T)
            w2p_s[:, j * 128:(j + 1) * 128] = _pk(w2t_s[:, j * 128:(j + 1) * 128])

        def load_o(t):
            return _up(ot_s[:, :, cols(t)].reshape(H * HP // 2, T))

        def h_rows(t, o, r0, r1):
            return xt_s[r0:r1, cols(t)].astype(f32) + _dot(_up(woT_s[r0 // 2:r1 // 2, :]), o)

        def tokens(x, by_half):
            n = x.shape[0] // 8
            if by_half:
                return [x[r * 8:r * 8 + 8, j * 128:(j + 1) * 128] for j in range(T // 128) for r in range(n)]
            return [x[r * 8:r * 8 + 8, 0:128] for r in range(n)]

        def scores_mxu(h, qt, c, buf):
            NOFF2 = ROH[h % 2] * NT
            MR2 = (S - NOFF2) // NT
            qw = qt_s[h, :, cols(qt)]
            rows = pl.ds((NOFF2 + c * MR2) // 2, MR2 // 2)
            if h % 2:
                kc = k_s[h // 2, rows, :]
                qw = jnp.concatenate([jnp.zeros((HP // 2, T), u32), qw], axis=0)
            else:
                kc = k_s[h // 2, rows, 0:HP]
            s = _dot(_up(kc), _up(qw))
            sbuf(buf)[pl.ds(NOFF2 + c * MR2, MR2), :] = s
            return tokens(s, False)[::QS], jnp.max(s.reshape(MR2 // 8, 8, T), axis=0)

        def scores_vpu(h, qt, c, buf, never, tk):
            sm = None
            RO2 = ROH[h % 2]
            nb = -(-RO2 // BR)
            for b in range(nb):
                r0 = c * RO2 + b * BR
                br = min(BR, RO2 - b * BR)
                acc = None
                for d in range(DH):
                    kb = kb2_s[(h - (H - HB)) * DH + d, pl.ds(r0 // 8, br // 8)]
                    qd = jnp.concatenate([jnp.broadcast_to(qf_s[h, qt * (T // 128) + j, d:d + 1, :], (8, 128))
                                          for j in range(T // 128)], axis=1)
                    if d % G2 == 0:
                        tok = tk[(b * DH + d) * len(tk) // (nb * DH)]
                        qd = jnp.where(never, jnp.concatenate([tok] * (T // 128), axis=1), qd)
                    t = jnp.concatenate([kb] * (T // 128), axis=2) * qd[None]
                    acc = t if acc is None else acc + t
                sbuf(buf)[pl.ds(r0, br), :] = acc.reshape(br, T)
                am = jnp.max(acc, axis=0)
                sm = am if sm is None else jnp.maximum(sm, am)
            return sm

        wo = wo_s[...].astype(f32)
        zrow = jnp.zeros((HP - DH, D), f32)
        wo = jnp.concatenate([p for h in range(H) for p in (wo[h * DH:(h + 1) * DH], zrow)], axis=0)
        woT_s[...] = _pk(wo.astype(bf16).T)
        b2c_s[...] = jnp.broadcast_to(b2_s[...].astype(f32).reshape(1, D), (128, D)).T

        one_rows = (lax.broadcasted_iota(jnp.int32, (16, T), 0) == 0).astype(f32)
        hid = {}
        outs = []
        st = {}

        def piece_a(t, pi, n):
            if pi == 0:
                st["o"] = load_o(t)
                st["h"] = []
            r0, r1 = pi * D // n, (pi + 1) * D // n
            att = _dot(_up(woT_s[r0 // 2:r1 // 2, :]), st["o"])
            st["h"].append(xt_s[r0:r1, cols(t)].astype(f32) + att)
            if pi == n - 1:
                hT = jnp.concatenate(st["h"], axis=0)
                if t == 0 and L0 is None:
                    hid[t] = (hT, _ln(hT, N2, extra=one_rows))
                else:
                    st["ln"] = (t, hT, _sum0(hT, N2) * (1.0 / D))
            return tokens(att, True)

        def centered(hT, mu, tk):
            mu8 = jnp.broadcast_to(mu, (8, T))
            n = D // LG
            parts = []
            for g in range(n):
                mg = jnp.where(z_s[0] > 0, jnp.concatenate([tk[g * len(tk) // n]] * (T // 128), axis=1), mu8)
                parts.append((hT[g * LG:(g + 1) * LG].reshape(LG // 8, 8, T) - mg[None]).reshape(LG, T))
            return jnp.concatenate(parts, axis=0)

        def ln_var(tk):
            t1, hT, mu = st["ln"]
            xc = centered(hT, mu, tk)
            st["ln"] = (t1, hT, mu, lax.rsqrt(_sum0(xc * xc, N2) * (1.0 / D) + EPS))

        def ln_out(tk):
            t1, hT, mu, r = st["ln"]
            hid[t1] = (hT, jnp.concatenate([centered(hT, mu, tk) * r, one_rows], axis=0).astype(bf16))

        def piece_w1(t, r0, r1):
            if r0 == 0:
                st["a"] = []
            a = _dot(_up(w1T_s[r0 // 2:r1 // 2, :]), hid[t][1])
            r = jnp.maximum(a, 0.0)
            st["a"].append((r0, r1, (r * r).astype(bf16)))
            return tokens(a, True)

        def piece_w2(t, k, n):
            r0, r1, a = st["a"][k]
            y = _dot(_up(w2p_s[:, r0:r1]), a)
            if k == 0:
                st["y"] = y + hid.pop(t)[0] + jnp.concatenate([b2c_s[...]] * (T // 128), axis=1)
            else:
                st["y"] = st["y"] + y
            if k == n - 1:
                cuts = LCUT if t == NT - 1 else (0, D)
                for a0, a1 in zip(cuts[:-1], cuts[1:]):
                    y_s[a0:a1, cols(t)] = st["y"][a0:a1].astype(bf16)
                    rs = pl.ds(a0, a1 - a0)
                    outs.append(pltpu.make_async_copy(y_s.at[rs, cols(t)], out_hbm.at[rs, cols(t)], sem.at[1]))
                    outs[-1].start()
            tk = tokens(y, False)
            if t + 1 < NT and k == KV:
                ln_var(tk)
            if t + 1 < NT and k == KN:
                ln_out(tk)
            return tk

        def chunk_pieces(t, n):
            ps = [(piece_w1, t, k * F // n, (k + 1) * F // n) for k in range(n)]
            if t + 1 < NT:
                na = 2 if n > 1 else 1
                ps += [(piece_a, t + 1, k, na) for k in range(na)]
            ps += [(piece_w2, t, k, n) for k in range(n)]
            return ps

        h14, h15 = H - 2, H - 1
        units = [(h14, 0), (h14, 1), (h15, 0), (h15, 1)] + [(h, q) for q in range(2, NT) for h in (h14, h15)]
        tot = len(units) * NT
        sched = {}
        sched[A0[0]] = [(piece_a, 0, 0, 2)]
        sched[A0[1]] = [(piece_a, 0, 1, 2)]
        rest = []
        for t in range(NT - 1):
            for k, pc in enumerate(chunk_pieces(t, 7)):
                if P0 + 16 * t + k < tot:
                    sched[P0 + 16 * t + k] = [pc]
                else:
                    rest.append(pc)
        rest += chunk_pieces(NT - 1, 1)

        never = z_s[0] > 0
        ms = {0: m}
        pend = [_up(p_s[j]) for j in range(LAG)]
        acc = None
        for i in range(tot):
            j = i + AHEAD
            s_now = None
            tk = None
            heavy = j < tot and j // NT >= FIRST
            if j < tot:
                h, qt = units[j // NT]
                if heavy:
                    qtk, sm = scores_mxu(h, qt, j % NT, j // NT)
                else:
                    s_now, sm = scores(h, h // 2, h % 2, qt, j % NT, never, (), j // NT)
            for pc in sched.get(i, []):
                tk = pc[0](*pc[1:])
            if L0 is not None and i == L0[0]:
                ln_var(tokens(s_now, False))
            if L0 is not None and i == L0[1]:
                ln_out(tokens(s_now, False))
            if j < tot:
                if heavy:
                    sm = jnp.maximum(sm, scores_vpu(h, qt, j % NT, j // NT, never, (qtk if QT else []) + tk))
                m8 = sm if m8 is None else jnp.maximum(m8, sm)
                if j % NT == NT - 1:
                    ms[j // NT] = jnp.max(m8, axis=0, keepdims=True)
                    m8 = None
            e = i + LAG
            if e < tot:
                if s_now is None and tk is not None and PG:
                    gs_ = [jnp.concatenate([tk[g * len(tk) // 2]] * (T // 128), axis=1) for g in range(2)]
                    s_now = jnp.concatenate([gs_[0]] * (MR // 16) + [gs_[1]] * (MR // 16), axis=0)
                pend.append(probs(e // NT, e % NT, ms[e // NT], s_now, never))
            h, qt = units[i // NT]
            o = _dot(_up(vt_s[h, :, cols(i % NT)]), pend.pop(0))
            acc = o if acc is None else acc + o
            if i % NT == NT - 1:
                ot_s[h, :, cols(qt)] = _pk((acc * pl.reciprocal(acc[DH:DH + 1], approx=False)).astype(bf16))
                acc = jnp.concatenate([jnp.zeros((HP - 8, T), f32),
                                       jnp.where(never, acc[HP - 8:HP], 0.0)], axis=0)
        for pc in rest:
            pc[0](*pc[1:])
        with scope("w_out"):
            for c in outs:
                c.wait()

    scratch = [
        pltpu.VMEM((H // 2, S // 2, 2 * HP), u32),
        pltpu.VMEM((H, HP // 2, S), u32),
        pltpu.VMEM((H, S // 128, HP, 128), f32),
        pltpu.VMEM((H, HP // 2, S), u32),
        pltpu.VMEM((H + 1, DH, NOFF // 8, 8, 128), f32),
        pltpu.VMEM((HB * DH, NOFF2 // 8, 8, 128), f32),
        pltpu.VMEM((H, HP // 2, S), u32),
        pltpu.VMEM((S, T), f32),
        pltpu.VMEM((S, T), f32),
        pltpu.VMEM((LAG, T // 2, T), u32),
        pltpu.VMEM((D, S), bf16),
        pltpu.VMEM((D, S), bf16),
        pltpu.VMEM((D, 3 * D), bf16),
        pltpu.VMEM((D, D), bf16),
        pltpu.VMEM((DA + 16, F), bf16),
        pltpu.VMEM((D, F), bf16),
        pltpu.VMEM((3 * D // 2, D), u32),
        pltpu.VMEM((D // 2, H * HP), u32),
        pltpu.VMEM((F // 2, DA), u32),
        pltpu.VMEM((D // 2, F), u32),
        pltpu.VMEM((D, 128), f32),
        pltpu.VMEM((H + 1, HP, NOFF), f32),
        pltpu.VMEM((NK2, 64, 128), f32),
        pltpu.VMEM((30 * 256,), bf16),
        pltpu.VMEM((D,), bf16),
        pltpu.SMEM((1,), jnp.int32),
        pltpu.SemaphoreType.DMA((6,)),
    ]
    return kern, scratch


def build(name="v45", **cfg):
    kern, scratch = make_kernel(**cfg)
    anyspec = pl.BlockSpec(memory_space=pl.ANY)

    @jax.jit
    def fn(A_x, A_wqkv, A_wo, B_x, B_w1, B_b1, B_w2, B_b2):
        xt = A_x.reshape(S, D).T
        out = pl.pallas_call(
            kern,
            out_shape=jax.ShapeDtypeStruct((D, S), bf16),
            in_specs=[anyspec] * 7,
            out_specs=anyspec,
            scratch_shapes=scratch,
            compiler_params=pltpu.CompilerParams(vmem_limit_bytes=110 * 1024 * 1024),
            name=name,
        )(xt, A_wqkv, A_wo, B_w1, B_b1, B_w2.T, B_b2)
        return out.T.reshape(1, S, D)
    return fn


_FN = build(name="fused_block")


@jax.jit
def pallas_sequential_preLN__mha_block__dense_activation_squared_relu__prompt_kernel(
    A_x: jax.Array,
    A_wqkv: jax.Array,
    A_wo: jax.Array,
    B_x: jax.Array,
    B_w1: jax.Array,
    B_b1: jax.Array,
    B_w2: jax.Array,
    B_b2: jax.Array,
):
    return _FN(A_x, A_wqkv, A_wo, B_x, B_w1, B_b1, B_w2, B_b2)
```

```python
import math

import jax
import jax.numpy as jnp
from jax import lax
import jax.experimental.pallas as pl
import jax.experimental.pallas.tpu as pltpu

bf16 = jnp.bfloat16
f32 = jnp.float32
u32 = jnp.uint32

S = 2048
D = 448
H = 16
DH = 28
HP = 32
F = 1792
EPS = 1e-5
QSCALE = (DH ** -0.5) * math.log2(math.e)

T = 256
NT = S // T
NL = T // 128
NI = NT * NT
DA = D + 16
RO = 16
RO_TAIL = (64, 80)
LAG = 2
AHEAD = NT + 2 + LAG
NV = 4
NOFF = RO * NT
NK2 = max(RO_TAIL) * NT // 128


def _pk(x):
    return pltpu.bitcast(x, u32)


def _up(x):
    return pltpu.bitcast(x, bf16)


def _dot(a, b):
    return jnp.dot(a, b, preferred_element_type=f32)


def _wide(x):
    return jnp.concatenate([x] * NL, axis=x.ndim - 1)


def _sum0(x, nch):
    parts = [x[i * 8:(i + 1) * 8] for i in range(x.shape[0] // 8)]
    accs = parts[:nch]
    for i in range(nch, len(parts)):
        accs[i % nch] = accs[i % nch] + parts[i]
    while len(accs) > 1:
        accs = [accs[i] + accs[i + 1] for i in range(0, len(accs), 2)]
    return jnp.sum(accs[0], axis=0, keepdims=True)


def _ln(x, nch):
    xc = x - _sum0(x, nch) * (1.0 / D)
    return xc * lax.rsqrt(_sum0(xc * xc, nch) * (1.0 / D) + EPS)


def _ln_chained(x, never):
    n = x.shape[1]
    mu = jnp.broadcast_to(_sum0(x, 2) * (1.0 / D), (8, n))
    accs = []
    for g in range(D // 32):
        mg = mu if g < 2 else jnp.where(never, accs[g - 2], mu)
        xc = x[g * 32:(g + 1) * 32].reshape(4, 8, n) - mg[None]
        sq = jnp.sum(xc * xc, axis=0)
        accs.append(sq if g == 0 else accs[-1] + sq)
    r = lax.rsqrt(jnp.sum(accs[-1], axis=0, keepdims=True) * (1.0 / D) + EPS)
    return (x - jnp.where(never, r, mu[0:1])) * r


def _lane_bcast(row, packed=False):
    if packed:
        row = jnp.concatenate([row, row], axis=0).astype(bf16)
        val = jnp.concatenate([row] * 8, axis=0).T.astype(f32)
    else:
        val = jnp.concatenate([row] * 16, axis=0).T
    return val.reshape(16, 8, 128)


def _kernel(xt_hbm, wqkv_hbm, wo_hbm, w1_hbm, b1_hbm, w2t_hbm, b2_hbm, out_hbm,
            k_s, qt_s, qf_s, vt_s, kb_s, kb2_s, ot_s, sA, sB, p_s, y_s,
            xt_s, wqkv_s, wo_s, w1_s, w2t_s, wqkvT_s, woT_s, w1T_s, w2p_s, b2c_s, ko_s, ko2_s,
            b1_s, b2_s, z_s, sem):
    def cols(t):
        return pl.ds(t * T, T)

    def colcp(src, dst, a, n, k):
        return pltpu.make_async_copy(src.at[:, pl.ds(a, n)], dst.at[:, pl.ds(a, n)], sem.at[k])

    cp_wv1 = colcp(wqkv_hbm, wqkv_s, 896, 256, 0)
    cp_xa = colcp(xt_hbm, xt_s, 0, T, 1)
    cp_wv2 = colcp(wqkv_hbm, wqkv_s, 1152, 192, 2)
    cp_xb = colcp(xt_hbm, xt_s, T, T, 2)
    cp_xc = colcp(xt_hbm, xt_s, 2 * T, (NV - 2) * T, 3)
    cp_wqk = colcp(wqkv_hbm, wqkv_s, 0, 896, 4)
    cp_xd = colcp(xt_hbm, xt_s, NV * T, S - NV * T, 5)
    late = [
        pltpu.make_async_copy(w1_hbm, w1_s.at[pl.ds(0, D)], sem.at[0]),
        pltpu.make_async_copy(wo_hbm, wo_s, sem.at[0]),
        pltpu.make_async_copy(w2t_hbm, w2t_s, sem.at[0]),
        pltpu.make_async_copy(b1_hbm, b1_s.at[pl.ds(0, F)], sem.at[0]),
        pltpu.make_async_copy(b2_hbm, b2_s, sem.at[0]),
    ]
    for c in (cp_wv1, cp_xa, cp_wv2, cp_xb, cp_xc, cp_wqk, cp_xd):
        c.start()
    z_s[0] = 0

    def get_never():
        return z_s[0] > 0

    ones_tail = (lax.broadcasted_iota(jnp.int32, (HP - DH, T), 0) == 0).astype(f32)
    zero_tail = jnp.zeros((HP - DH, T), f32)

    def wT(a, b):
        wqkvT_s[a // 2:b // 2, :] = _pk(wqkv_s[:, a:b].T)

    def ln1(t):
        return _ln_chained(xt_s[:, cols(t)].astype(f32), get_never()).astype(bf16)

    ktoks = []

    def proj_k(t, xn):
        kk = _dot(_up(wqkvT_s[D // 2:D, :]), xn)
        for g in range(H // 2):
            ka = jnp.concatenate([kk[2 * g * DH:(2 * g + 1) * DH], zero_tail], axis=0)
            kb = jnp.concatenate([kk[(2 * g + 1) * DH:(2 * g + 2) * DH], zero_tail], axis=0)
            if t == 0:
                ko_s[2 * g] = ka[:, 0:NOFF]
                ko_s[2 * g + 1] = kb[:, 0:NOFF]
            kt = _pk(jnp.concatenate([ka, kb], axis=0).astype(bf16).T)
            k_s[g, pl.ds(t * T // 2, T // 2), :] = kt
            if t == NT - 1 and g > 0:
                tk = pltpu.bitcast(kt[T // 2 - 8:T // 2], f32)
                ktoks.append(jnp.concatenate([tk] * 4, axis=1))
        if t == 0:
            ko_s[H] = jnp.zeros((HP, NOFF), f32)
        for j in range(NL):
            if t * NL + j < NK2:
                ko2_s[t * NL + j] = kk[D - 64:D, j * 128:(j + 1) * 128]

    def proj_v(t, xn, ha=0, hb=H):
        vv = _dot(_up(wqkvT_s[D + ha * DH // 2:D + hb * DH // 2, :]), xn)
        for h in range(ha, hb):
            v = jnp.concatenate([vv[(h - ha) * DH:(h - ha + 1) * DH], ones_tail], axis=0)
            vt_s[h, :, cols(t)] = _pk(v.astype(bf16))
        return vv

    def proj_q(t, xn):
        qq = _dot(_up(wqkvT_s[0:D // 2, :]), xn) * QSCALE
        for h in range(H):
            q = jnp.concatenate([qq[h * DH:(h + 1) * DH], zero_tail], axis=0)
            qt_s[h, :, cols(t)] = _pk(q.astype(bf16))
            for j in range(NL):
                qf_s[h, t * NL + j] = q[:, j * 128:(j + 1) * 128]

    def kb_make(h, d, gate=None):
        row = jnp.broadcast_to(ko_s[h, d:d + 1, :], (8, NOFF))
        if gate is not None:
            row = jnp.where(get_never(), gate, row)
        val = _lane_bcast(row, packed=gate is not None)
        kb_s[h, d] = val
        return val[15]

    def kb2_make(r, j):
        val = _lane_bcast(jnp.broadcast_to(ko2_s[j, pl.ds(64 - 2 * DH + r, 1), :], (8, 128)))
        kb2_s[r, pl.ds(j * 16, 16)] = val
        return val[15]

    xn = {}
    cp_wv1.wait()
    wT(896, 1152)
    cp_xa.wait()
    xn[0] = jnp.concatenate([_ln(xt_s[:, j * 128:(j + 1) * 128].astype(f32), 4).astype(bf16)
                             for j in range(NL)], axis=1)
    proj_v(0, xn[0], 0, 4)
    cp_wv2.wait()
    cp_xb.wait()
    wT(1152, 1344)
    xn[1] = ln1(1)
    proj_v(0, xn[0], 4, 8)
    proj_v(0, xn[0], 8, H)
    proj_v(1, xn[1], 0, 8)
    cp_xc.wait()
    xn[2] = ln1(2)
    proj_v(1, xn[1], 8, H)
    for t in range(2, NV - 1):
        xn[t + 1] = ln1(t + 1)
        proj_v(t, xn[t])
    proj_v(NV - 1, xn[NV - 1], 0, 8)
    cp_wqk.wait()
    wT(384, 896)
    wT(0, 384)
    proj_v(NV - 1, xn[NV - 1], 8, H)
    for t in range(NV):
        proj_k(t, xn[t])
        if t > 0:
            proj_q(t - 1, xn[t - 1])
    for c in late:
        c.start()
    cp_xd.wait()
    xn[NV] = ln1(NV)
    proj_q(NV - 1, xn[NV - 1])
    todo = [(h, d) for h in range(3) for d in range(DH)]
    for t in range(NV, NT):
        proj_k(t, xn[t])
        if t + 1 < NT:
            xn[t + 1] = ln1(t + 1)
        vv = proj_v(t, xn[t])
        now, todo = todo[:42], todo[42:]
        for k, (h, d) in enumerate(now):
            half, tr = divmod(k * 2 * (D // 8) // len(now), D // 8)
            kb_make(h, d, vv[tr * 8:tr * 8 + 8, half * 128:(half + 1) * 128])
        proj_q(t, xn[t])

    def sbuf(u):
        return sA if u % 2 == 0 else sB

    def scores_mxu(h, g, odd, qt, c, u, ro):
        mr = T - ro
        r0 = ro * NT + c * mr
        qw = qt_s[h, :, cols(qt)]
        if odd:
            kc = k_s[g, pl.ds(r0 // 2, mr // 2), :]
            qw = jnp.concatenate([jnp.zeros((HP // 2, T), u32), qw], axis=0)
        else:
            kc = k_s[g, pl.ds(r0 // 2, mr // 2), 0:HP]
        s = _dot(_up(kc), _up(qw))
        sbuf(u)[pl.ds(r0, mr), :] = s
        return s, jnp.max(s.reshape(mr // 8, 8, T), axis=0)

    def scores_vpu(h, qt, r0, n, u, kb_row, gate, never):
        acc = None
        for d in range(DH):
            qd = jnp.concatenate([jnp.broadcast_to(qf_s[h, qt * NL + j, d:d + 1, :], (8, 128))
                                  for j in range(NL)], axis=1)
            if d % 3 == 0:
                qd = jnp.where(never, gate(d), qd)
            t = _wide(kb_row(d, pl.ds(r0 // 8, n // 8))) * qd[None]
            acc = t if acc is None else acc + t
        sbuf(u)[pl.ds(r0, n), :] = acc.reshape(n, T)
        return jnp.max(acc, axis=0)

    def scores(h, g, odd, qt, c, u, never, toks=()):
        s, sm = scores_mxu(h, g, odd, qt, c, u, RO)

        def gate(d):
            tr = d * (T - RO) // DH // 8 * 8
            x = s[tr:tr + 8]
            for tok in (toks if d == 0 else ()):
                x = jnp.maximum(x, tok)
            return x
        sv = scores_vpu(h, qt, c * RO, RO, u, lambda d, rows: kb_s[h, d, rows], gate, never)
        return [s[0:8], s[(T - RO) // 2:(T - RO) // 2 + 8]], jnp.maximum(sm, sv)

    def probs(u, c, m, gates, never, toks=()):
        s_ref = sbuf(u)
        if gates is None:
            return jnp.exp2(s_ref[cols(c), :] - m).astype(bf16)
        m8 = jnp.broadcast_to(m, (8, T))
        parts = []
        for g, gate in enumerate(gates):
            if g == 0 and toks:
                left = gate[:, 0:128]
                for tok in toks:
                    left = jnp.maximum(left, tok)
                gate = jnp.concatenate([left, gate[:, 128:]], axis=1)
            s = s_ref[pl.ds(c * T + g * 128, 128), :].reshape(16, 8, T)
            parts.append((s - jnp.where(never, gate, m8)[None]).reshape(128, T))
        return jnp.exp2(jnp.concatenate(parts, axis=0)).astype(bf16)

    def pv_step(h, qt, c, p, acc, never):
        o = _dot(_up(vt_s[h, :, cols(c)]), p)
        acc = o if acc is None else acc + o
        if c == NT - 1:
            ot_s[h, :, cols(qt)] = _pk((acc * pl.reciprocal(acc[DH:DH + 1], approx=False)).astype(bf16))
            acc = jnp.concatenate([jnp.zeros((HP - 8, T), f32),
                                   jnp.where(never, acc[HP - 8:HP], 0.0)], axis=0)
        return acc

    def fold_max(j, sm, m8, ms):
        m8 = sm if m8 is None else jnp.maximum(m8, sm)
        if j % NT == NT - 1:
            ms[j // NT] = jnp.max(m8, axis=0, keepdims=True)
            m8 = None
        return m8

    never = get_never()
    m8 = None
    ms = {}
    for j in range(AHEAD):
        gates, sm = scores(0, 0, 0, j // NT, j % NT, j // NT, never, ktoks if j == 0 else ())
        m8 = fold_max(j, sm, m8, ms)
        if j >= AHEAD - LAG:
            p_s[j - (AHEAD - LAG)] = _pk(probs(0, j - (AHEAD - LAG), ms[0], gates, never))

    jobs2 = [(hh, r, j) for r in range(4) for hh in range(2) for j in range(RO_TAIL[hh] * NT // 128)]

    def body(g0, carry):
        m, m8 = carry
        never = get_never()
        hs = [2 * g0 + k for k in range(5)]
        gs = [g0, g0 + 1]
        ms = {0: m}
        toks = {}
        pend = [_up(p_s[j]) for j in range(LAG)]
        acc = None
        for i in range(2 * NI):
            j = i + AHEAD
            hh, jj = divmod(j, NI)
            gates, sm = scores(hs[hh], gs[hh // 2], hh % 2, jj // NT, jj % NT, j // NT, never)
            m8 = fold_max(j, sm, m8, ms)
            k = (i - 3) // 2
            if i % 2 == 1 and 0 <= k < 2 * DH:
                toks[i + 3] = [kb_make(hs[3 + k // DH], k % DH)]
            k = (i - 4) // 2
            if i % 2 == 0 and 0 <= k < len(jobs2):
                toks[i + 3] = [kb2_make(g0 * 4 + jobs2[k][0] * DH + jobs2[k][1], jobs2[k][2])]
            e = i + LAG
            pend.append(probs(e // NT, e % NT, ms[e // NT], gates, never, toks.get(i, ())))
            hh, ii = divmod(i, NI)
            acc = pv_step(hs[hh], ii // NT, ii % NT, pend.pop(0), acc, never)
        for j in range(LAG):
            p_s[j] = _pk(pend[j])
        return ms[2 * NT], m8

    m, m8 = lax.fori_loop(0, H // 2 - 1, body, (ms[0], m8))

    for c in late:
        c.wait()
    b1 = jnp.broadcast_to(b1_s[pl.ds(0, F)].astype(f32).reshape(1, F), (DA - D, F))
    first_row = lax.broadcasted_iota(jnp.int32, (DA - D, F), 0) == 0
    w1_s[D:DA, :] = jnp.where(first_row, b1, 0.0).astype(bf16)
    for j in range(F // 128):
        w1T_s[j * 64:(j + 1) * 64, :] = _pk(w1_s[0:DA, j * 128:(j + 1) * 128].T)
        w2p_s[:, j * 128:(j + 1) * 128] = _pk(w2t_s[:, j * 128:(j + 1) * 128])
    wo = wo_s[...].astype(f32)
    zrow = jnp.zeros((HP - DH, D), f32)
    wo = jnp.concatenate([p for h in range(H) for p in (wo[h * DH:(h + 1) * DH], zrow)], axis=0)
    woT_s[...] = _pk(wo.astype(bf16).T)
    b2c_s[...] = jnp.broadcast_to(b2_s[...].astype(f32).reshape(1, D), (128, D)).T

    never = get_never()
    one_rows = (lax.broadcasted_iota(jnp.int32, (DA - D, T), 0) == 0).astype(f32)
    hid = {}
    outs = []
    st = {}

    def tokens(x, by_half):
        n = x.shape[0] // 8

        def tk(a, b):
            j, r = divmod(a * n * (NL if by_half else 1) // b, n)
            return _wide(x[r * 8:r * 8 + 8, j * 128:(j + 1) * 128])
        return tk

    def with_ones(y):
        return jnp.concatenate([y, one_rows], axis=0).astype(bf16)

    def centered(hT, mu, tk):
        mu8 = jnp.broadcast_to(mu, (8, T))
        n = D // 32
        parts = []
        for g in range(n):
            mg = jnp.where(never, tk(g, n), mu8)
            parts.append((hT[g * 32:(g + 1) * 32].reshape(4, 8, T) - mg[None]).reshape(32, T))
        return jnp.concatenate(parts, axis=0)

    def piece_wo(t, k, n):
        if k == 0:
            st["h"] = []
        r0, r1 = k * D // n, (k + 1) * D // n
        att = _dot(_up(woT_s[r0 // 2:r1 // 2, :]), _up(ot_s[:, :, cols(t)].reshape(H * HP // 2, T)))
        st["h"].append(xt_s[r0:r1, cols(t)].astype(f32) + att)
        if k == n - 1:
            hT = jnp.concatenate(st["h"], axis=0)
            if t == 0:
                hid[t] = (hT, with_ones(_ln(hT, 2)))
            else:
                st["ln"] = (hT, _sum0(hT, 2) * (1.0 / D))
        return tokens(att, True)

    def piece_w1(t, k, n):
        if k == 0:
            st["a"] = []
        r0, r1 = k * F // n, (k + 1) * F // n
        a = jnp.maximum(_dot(_up(w1T_s[r0 // 2:r1 // 2, :]), hid[t][1]), 0.0)
        a = a * a
        st["a"].append(a.astype(bf16))
        return tokens(a, True)

    def piece_w2(t, k, n):
        y = _dot(_up(w2p_s[:, k * F // n:(k + 1) * F // n]), st["a"][k])
        st["y"] = y + hid.pop(t)[0] + _wide(b2c_s[...]) if k == 0 else st["y"] + y
        if k == n - 1:
            cuts = (0, 224, 352, D) if t == NT - 1 else (0, D)
            for r0, r1 in zip(cuts[:-1], cuts[1:]):
                y_s[r0:r1, cols(t)] = st["y"][r0:r1].astype(bf16)
                rs = pl.ds(r0, r1 - r0)
                outs.append(pltpu.make_async_copy(y_s.at[rs, cols(t)], out_hbm.at[rs, cols(t)], sem.at[1]))
                outs[-1].start()
        tk = tokens(y, False)
        if t + 1 < NT and k == 1:
            hT, mu = st["ln"]
            xc = centered(hT, mu, tk)
            st["ln"] = (hT, mu, lax.rsqrt(_sum0(xc * xc, 2) * (1.0 / D) + EPS))
        if t + 1 < NT and k == 4:
            hT, mu, r = st["ln"]
            hid[t + 1] = (hT, with_ones(centered(hT, mu, tk) * r))
        return tk

    pieces = []
    for t in range(NT - 1):
        pieces += [(piece_w1, t, k, 7) for k in range(7)]
        pieces += [(piece_wo, t + 1, k, 2) for k in range(2)]
        pieces += [(piece_w2, t, k, 7) for k in range(7)]
    pieces += [(piece_w1, NT - 1, 0, 1), (piece_w2, NT - 1, 0, 1)]

    ha, hb = H - 2, H - 1
    units = [(ha, 0), (ha, 1), (hb, 0), (hb, 1)] + [(h, q) for q in range(2, NT) for h in (ha, hb)]
    tot = len(units) * NT
    start = 5 * NT - AHEAD
    ms = {0: m}
    pend = [_up(p_s[j]) for j in range(LAG)]
    acc = None
    for i in range(tot):
        j = i + AHEAD
        gates = None
        if j < tot:
            h, qt = units[j // NT]
            if i < start:
                gates, sm = scores(h, h // 2, h % 2, qt, j % NT, j // NT, never)
            else:
                ro = RO_TAIL[h - ha]
                _, sm = scores_mxu(h, h // 2, h % 2, qt, j % NT, j // NT, ro)
        if i == 3 * NT:
            piece_wo(0, 0, 1)
        if i >= start:
            pc = pieces.pop(0)
            tk = pc[0](*pc[1:])
            gates = [tk(0, 2), tk(1, 2)]
            if j < tot:
                nb = -(-ro // 32)
                for b in range(nb):
                    sv = scores_vpu(h, qt, j % NT * ro + b * 32, min(32, ro - b * 32), j // NT,
                                    lambda d, rows: kb2_s[(h - ha) * DH + d, rows],
                                    lambda d: tk(b * DH + d, nb * DH), never)
                    sm = jnp.maximum(sm, sv)
        if j < tot:
            m8 = fold_max(j, sm, m8, ms)
        e = i + LAG
        if e < tot:
            pend.append(probs(e // NT, e % NT, ms[e // NT], gates, never))
        h, qt = units[i // NT]
        acc = pv_step(h, qt, i % NT, pend.pop(0), acc, never)
    for pc in pieces:
        pc[0](*pc[1:])
    for c in outs:
        c.wait()


_SCRATCH = [
    pltpu.VMEM((H // 2, S // 2, 2 * HP), u32),
    pltpu.VMEM((H, HP // 2, S), u32),
    pltpu.VMEM((H, S // 128, HP, 128), f32),
    pltpu.VMEM((H, HP // 2, S), u32),
    pltpu.VMEM((H + 1, DH, NOFF // 8, 8, 128), f32),
    pltpu.VMEM((2 * DH, NK2 * 16, 8, 128), f32),
    pltpu.VMEM((H, HP // 2, S), u32),
    pltpu.VMEM((S, T), f32),
    pltpu.VMEM((S, T), f32),
    pltpu.VMEM((LAG, T // 2, T), u32),
    pltpu.VMEM((D, S), bf16),
    pltpu.VMEM((D, S), bf16),
    pltpu.VMEM((D, 3 * D), bf16),
    pltpu.VMEM((D, D), bf16),
    pltpu.VMEM((DA + 16, F), bf16),
    pltpu.VMEM((D, F), bf16),
    pltpu.VMEM((3 * D // 2, D), u32),
    pltpu.VMEM((D // 2, H * HP), u32),
    pltpu.VMEM((F // 2, DA), u32),
    pltpu.VMEM((D // 2, F), u32),
    pltpu.VMEM((D, 128), f32),
    pltpu.VMEM((H + 1, HP, NOFF), f32),
    pltpu.VMEM((NK2, 64, 128), f32),
    pltpu.VMEM((30 * 256,), bf16),
    pltpu.VMEM((D,), bf16),
    pltpu.SMEM((1,), jnp.int32),
    pltpu.SemaphoreType.DMA((6,)),
]


@jax.jit
def pallas_sequential_preLN__mha_block__dense_activation_squared_relu__prompt_kernel(
    A_x: jax.Array,
    A_wqkv: jax.Array,
    A_wo: jax.Array,
    B_x: jax.Array,
    B_w1: jax.Array,
    B_b1: jax.Array,
    B_w2: jax.Array,
    B_b2: jax.Array,
):
    del B_x
    hbm = pl.BlockSpec(memory_space=pl.ANY)
    out = pl.pallas_call(
        _kernel,
        out_shape=jax.ShapeDtypeStruct((D, S), bf16),
        in_specs=[hbm] * 7,
        out_specs=hbm,
        scratch_shapes=_SCRATCH,
        compiler_params=pltpu.CompilerParams(vmem_limit_bytes=110 * 1024 * 1024),
        name="preln_block",
    )(A_x.reshape(S, D).T, A_wqkv, A_wo, B_w1, B_b1, B_w2.T, B_b2)
    return out.T.reshape(1, S, D)
```
